```python
import jax
import jax.numpy as jnp

def _softmax(x, axis=-1):
    return jax.nn.softmax(x, axis=axis)
def _gelu(x):
    return jax.nn.gelu(x, approximate=True)
def _silu(x):
    return jax.nn.silu(x)
def _sigmoid(x):
    return jax.nn.sigmoid(x)
def _layernorm(x, axis=-1, eps=1e-5):
    m = jnp.mean(x, axis=axis, keepdims=True)
    v = jnp.var(x, axis=axis, keepdims=True)
    return (x - m) / jnp.sqrt(v + eps)
def _scatter_add(tgt, idx, src, axis=0):
    return tgt.at[idx].add(src)
def _segment_sum(src, seg, n):
    return jax.ops.segment_sum(src, seg, n)
class _Rng:
    def __init__(self, key):
        self._k = key
    def _next(self):
        self._k, sub = jax.random.split(self._k)
        return sub
    def normal(self, shape):
        return jax.random.normal(self._next(), shape, dtype=jnp.bfloat16)
    def randint(self, lo, hi, shape):
        return jax.random.randint(self._next(), shape, lo, hi, dtype=jnp.int32)
    def uniform(self, shape, lo=0.0, hi=1.0):
        return jax.random.uniform(self._next(), shape, jnp.bfloat16, lo, hi)
    def permutation(self, n):
        return jax.random.permutation(self._next(), n)


kernel_name = 'interleave_layers__sliding_block_cached__dense_activation_gelu__decode'

def setup_inputs():
    _rng = _Rng(jax.random.key(int.from_bytes(__import__("os").urandom(4), "little")))
    _w = (lambda a: (lambda t: t.astype(jnp.bfloat16) if jnp.issubdtype(t.dtype, jnp.floating) else t)(jnp.asarray(a)))
    def _A_setup():
        B, Sq, D = 1, 1, 640
        Hq, Hkv, Sk, Dh = 32, 32, 32768, 192
        assert Hq % Hkv == 0, (Hq, Hkv)
        return {
            "x": _w((lambda *s: _rng.normal(s) * 0.05)(B, Sq, D)),
            "k_cache": _w((lambda *s: _rng.normal(s) * 0.05)(B, Hkv, Sk, Dh)),
            "v_cache": _w((lambda *s: _rng.normal(s) * 0.05)(B, Hkv, Sk, Dh)),
            "wq": _w((lambda *s: _rng.normal(s) * 0.05)(D, Hq * Dh) * (D ** -0.5)),
            "wo": _w((lambda *s: _rng.normal(s) * 0.05)(Hq * Dh, D) * ((Hq * Dh) ** -0.5)),
        }
    _A_in = _A_setup()

    def _B_setup():
        B, S, D, F = 1, 1, 640, 1536
        return {
            "x": _w((lambda *s: _rng.normal(s) * 0.05)(B, S, D)),
            "w1": _w((lambda *s: _rng.normal(s) * 0.05)(D, F) * (D ** -0.5)),
            "b1": _w((lambda *s: _rng.normal(s) * 0.05)(F) * 0.01),
            "w2": _w((lambda *s: _rng.normal(s) * 0.05)(F, D) * (F ** -0.5)),
            "b2": _w((lambda *s: _rng.normal(s) * 0.05)(D) * 0.01),
        }
    _B_in = _B_setup()

    return {
        "A_x": _A_in["x"],
        "A_k_cache": _A_in["k_cache"],
        "A_v_cache": _A_in["v_cache"],
        "A_wq": _A_in["wq"],
        "A_wo": _A_in["wo"],
        "B_x": _B_in["x"],
        "B_w1": _B_in["w1"],
        "B_b1": _B_in["b1"],
        "B_w2": _B_in["w2"],
        "B_b2": _B_in["b2"],
    }

def reference(A_x, A_k_cache, A_v_cache, A_wq, A_wo, B_x, B_w1, B_b1, B_w2, B_b2):
    def _A_ref(x, k_cache, v_cache, wq, wo):
        B, Sq, D = x.shape
        Hq, Dh = 32, 192
        Hkv, Sk = k_cache.shape[1], k_cache.shape[2]
        W = min(4096, max(256, Sk // 4))
        rep = Hq // Hkv
        q = (lambda x, *d: x.transpose(*d))((x @ wq).reshape(B, Sq, Hq, Dh), 0, 2, 1, 3)
        k = jnp.repeat(k_cache[:, :, Sk - W:, :], rep, axis=1)
        v = jnp.repeat(v_cache[:, :, Sk - W:, :], rep, axis=1)
        scores = jnp.einsum("bhqd,bhkd->bhqk", q, k) * (Dh ** -0.5)
        p = _softmax(scores, axis=-1)
        o = jnp.einsum("bhqk,bhkd->bhqd", p, v)
        return (lambda x, *d: x.transpose(*d))(o, 0, 2, 1, 3).reshape(B, Sq, Hq * Dh) @ wo

    def _B_ref(x, w1, b1, w2, b2):
        h = jnp.einsum("bsd,df->bsf", x, w1) + b1
        h = _gelu(h)
        return jnp.einsum("bsf,fd->bsd", h, w2) + b2

    x = A_x
    x = x + _A_ref(_layernorm(x, axis=-1), A_k_cache, A_v_cache, A_wq, A_wo)
    x = x + _B_ref(_layernorm(x, axis=-1), B_w1, B_b1, B_w2, B_b2)
    x = x + _A_ref(_layernorm(x, axis=-1), A_k_cache, A_v_cache, A_wq, A_wo)
    x = x + _B_ref(_layernorm(x, axis=-1), B_w1, B_b1, B_w2, B_b2)
    return x
```

```python
import jax
import jax.numpy as jnp
from jax import lax
import jax.experimental.pallas as pl
import jax.experimental.pallas.tpu as pltpu

D, F, H, DH, SK, W = 640, 1536, 32, 192, 32768, 4096
NS = H * DH // 8
GS = 96
NG = NS // GS
NJ = W // 256
WIN0 = (SK - W) // 16
WROWS = W // 16
SPLIT = 192
DRAIN_MXU_U = 3
EPS = 1e-5
F32, BF16, I32 = jnp.float32, jnp.bfloat16, jnp.int32
NN = (((1,), (0,)), ((), ()))
NT = (((1,), (1,)), ((), ()))


def _tile_order(a, rows):
    r, c = a.shape
    a = a.reshape(r // 8, 8, c // 128, 128).transpose(0, 2, 1, 3)
    return a.reshape(-1, rows, 128)


def _rnd(x):
    return x.astype(BF16).astype(F32)


def _rhs(words):
    return pltpu.bitcast(words.reshape(-1, 128), BF16)


def _kernel(x_hbm, k_hbm, v_hbm, wq_hbm, wo_hbm, w1_hbm, b1_hbm, w2_hbm, b2_hbm,
            out_ref,
            kb, vb, wqb, wob, w1b, w2b, xb, b1b, b2b,
            ylhs, qlhs, pbuf, olhs, oacc, sems, ksem, vsem, osem):
    kw, vw = kb.bitcast(I32), vb.bitcast(I32)
    wqw, wow = wqb.bitcast(I32), wob.bitcast(I32)
    w1w, w2w = w1b.bitcast(I32), w2b.bitcast(I32)

    sub = lax.broadcasted_iota(I32, (8, 128), 0)
    lane = lax.broadcasted_iota(I32, (8, 128), 1)

    def issue_kv(src, dst, sem, g):
        def body(t, c):
            s = g * GS + 2 * t
            for r0, n, prio in ((0, SPLIT, 1), (SPLIT, WROWS - SPLIT, 0)):
                pltpu.make_async_copy(
                    src.at[pl.ds(s, 2), pl.ds(WIN0 + r0, n), :],
                    dst.at[pl.ds(s, 2), pl.ds(r0, n), :], sem.at[g]).start(priority=prio)
            return c
        lax.fori_loop(0, GS // 2, body, 0)

    def issue_w(src, dst, sem, start, count, unit):
        big = unit * 3 // 4

        def body(t, c):
            s = start + unit * t
            for r0, n, prio in ((0, big, 1), (big, unit - big, 0)):
                pltpu.make_async_copy(src.at[pl.ds(s + r0, n)], dst.at[pl.ds(s + r0, n)],
                                      sem).start(priority=prio)
            return c
        lax.fori_loop(0, count // unit, body, 0)

    def issue_wq():
        def body(t, c):
            for r0, n, prio in ((0, 288, 1), (288, 96, 0)):
                pltpu.make_async_copy(wq_hbm.at[t, pl.ds(r0, n), :], wqb.at[t, pl.ds(r0, n), :],
                                      sems.at[0]).start(priority=prio)
            return c
        lax.fori_loop(0, 80, body, 0)

    def wait(ref, sem):
        pltpu.make_async_copy(ref, ref, sem).wait()

    def bcast_row(v, r):
        return jnp.broadcast_to(v[r:r + 1, :], (8, 128))

    def halves(v):
        rolled = pltpu.roll(v, 4, 0)
        return jnp.where(sub < 4, v, rolled), jnp.where(sub < 4, rolled, v)

    def all_rows_sum(v):
        return jnp.broadcast_to(jnp.sum(v, axis=0, keepdims=True), (8, 128))

    def gather(v, idx):
        return jnp.take_along_axis(v, idx, axis=1)

    same_c = ((lane >> 3) & 1) == (sub >> 2)

    def expand(v, half):
        return gather(v, 64 * half + ((lane >> 4) << 3) + (lane & 7))

    def head_mask(t):
        return same_c & ((sub & 3) == (8 * t) // 24)

    def down_lhs(v):
        idx = (lane & ~8) + ((sub & 2) << 2)
        return jnp.where(same_c, gather(v, idx), 0.0)

    def layernorm_to_lhs(xs):
        tot = xs[0] + xs[1] + xs[2] + xs[3] + xs[4]
        mean = jnp.sum(tot, axis=1, keepdims=True) * (1.0 / D)
        ds = [x - mean for x in xs]
        sq = ds[0] * ds[0] + ds[1] * ds[1] + ds[2] * ds[2] + ds[3] * ds[3] + ds[4] * ds[4]
        var = jnp.sum(sq, axis=1, keepdims=True) * (1.0 / D)
        inv = 1.0 / jnp.sqrt(var + EPS)
        for t in range(10):
            ylhs[t] = jnp.where(same_c, _rnd(expand(ds[t // 2], t % 2) * inv), 0.0)

    def up_proj(ww, j):
        y = jnp.concatenate([ylhs[t] for t in range(10)], axis=1)
        return lax.dot_general(y, _rhs(ww[:, pl.ds(j * 8, 8), :]), NN, preferred_element_type=F32)

    def down_proj(ww, u0, lhs):
        n = len(lhs)
        a = jnp.concatenate(lhs, axis=1)
        return [lax.dot_general(a, _rhs(ww[pl.ds(u0, 8 * n), 8 * t:8 * t + 8, :]), NN,
                                preferred_element_type=F32) for t in range(5)]

    def collect(outs):
        res = []
        for n in range(5):
            a, b = n, n + 5
            res.append(bcast_row(outs[a // 2], 4 * (a % 2)) + bcast_row(outs[b // 2], 4 * (b % 2) + 2))
        return res

    def q_proj(g, slot):
        for jj in range(3):
            off = pl.multiple_of((3 * g + jj) * 8, 8)
            y = jnp.concatenate([ylhs[t] for t in range(10)], axis=1)
            q = lax.dot_general(y, _rhs(wqw[:, pl.ds(off, 8), :]), NN, preferred_element_type=F32)
            for c, qc in enumerate(halves(_rnd(q))):
                for half in range(2):
                    t = 4 * jj + 2 * c + half
                    qlhs[slot, t] = jnp.where(head_mask(t), expand(qc, half), 0.0)

    def scores(g, slot):
        q = jnp.concatenate([qlhs[slot, t] for t in range(12)], axis=1)
        return [lax.dot_general(q, _rhs(kw[pl.ds(g * GS, GS), 8 * j:8 * j + 8, :]), NN,
                                preferred_element_type=F32) for j in range(NJ)]

    def softmax(ss, slot):
        ss = [s * (DH ** -0.5) for s in ss]
        m = ss[0]
        for s in ss[1:]:
            m = jnp.maximum(m, s)
        m = jnp.maximum(m, pltpu.roll(m, 4, 0))
        m = jnp.max(m, axis=1, keepdims=True)
        es = [jnp.exp(s - m) for s in ss]
        l = es[0]
        for e in es[1:]:
            l = l + e
        l = l + pltpu.roll(l, 4, 0)
        inv = 1.0 / jnp.sum(l, axis=1, keepdims=True)
        for j in range(NJ):
            pbuf[slot, j] = _rnd(es[j] * inv)

    def pv_mxu(g, slot, u0, u1):
        acc = None
        for j in range(NJ):
            r = lax.dot_general(pbuf[slot, j],
                                _rhs(vw[pl.ds(g * GS + 16 * u0, 16 * (u1 - u0)), 8 * j:8 * j + 8, :]),
                                NT, preferred_element_type=F32)
            acc = r if acc is None else acc + r
        idx = ((lane & 48) << 1) + ((sub & 2) << 3) + (lane & 7)
        for u in range(u0, u1):
            parts = []
            for t in (2 * u, 2 * u + 1):
                a = acc[:, 128 * (t - 2 * u0):128 * (t - 2 * u0 + 1)]
                a = all_rows_sum(jnp.where(head_mask(t), a, 0.0))
                parts.append(gather(a, idx) + gather(a, idx + 8))
            olhs[u] = jnp.where(same_c, _rnd(jnp.where(lane < 64, parts[0], parts[1])), 0.0)

    def pv_vpu(g, slot, u0, u1):
        diag = lane - (((sub & 3) << 1) + (sub >> 2))
        p, cur = None, -1
        for u in range(u0, u1):
            col = jnp.zeros((8, 128), F32)
            for i in range(16):
                s = 16 * u + i
                if s // 24 != cur:
                    cur = s // 24
                    p = [jnp.take_along_axis(pbuf[slot, j], (sub & 4) + cur, axis=0)
                         for j in range(NJ)]
                lo = hi = None
                for j in range(NJ):
                    w = vw[g * GS + s, 8 * j:8 * j + 8, :]
                    a = pltpu.bitcast(w << 16, F32) * p[j]
                    b = pltpu.bitcast(w & -65536, F32) * p[j]
                    lo = a if lo is None else lo + a
                    hi = b if hi is None else hi + b
                z = jnp.where(sub < 4, lo, hi) + pltpu.roll(jnp.where(sub < 4, hi, lo), 4, 0)
                col = jnp.where(diag == 8 * i, jnp.sum(z, axis=1, keepdims=True), col)
            olhs[u] = down_lhs(_rnd(all_rows_sum(col)))

    def o_proj(g):
        outs = down_proj(wow, g * 48, [olhs[u] for u in range(6)])
        for t in range(5):
            oacc[t] += outs[t]

    def ffn(xs, before_w1, before_w2):
        layernorm_to_lhs(xs)
        before_w1()
        b1 = b1b[...].astype(F32)
        lhs = []
        for j in range(6):
            bias = jnp.where(sub < 4, bcast_row(b1, 2 * j), bcast_row(b1, 2 * j + 1))
            h = jax.nn.gelu(up_proj(w1w, j) + bias, approximate=True)
            lhs += [down_lhs(v) for v in halves(_rnd(h))]
        before_w2()
        b2 = b2b[...].astype(F32)
        ys = collect(down_proj(w2w, 0, lhs))
        return [xs[n] + ys[n] + bcast_row(b2, n) for n in range(5)]

    def add_attn(xs):
        ys = collect([oacc[t] for t in range(5)])
        return [xs[n] + ys[n] for n in range(5)]

    def zero_oacc():
        for t in range(5):
            oacc[t] = jnp.zeros((8, 128), F32)

    small = [pltpu.make_async_copy(s, d, sems.at[3 + i])
             for i, (s, d) in enumerate(((x_hbm, xb), (b1_hbm, b1b), (b2_hbm, b2b)))]
    for c in small:
        c.start()
    issue_wq()
    issue_kv(k_hbm, kb, ksem, 0)
    for c in small:
        c.wait()
    x0 = xb[...].astype(F32)
    xs = [jnp.broadcast_to(x0[:, 128 * n:128 * n + 128], (8, 128)) for n in range(5)]
    layernorm_to_lhs(xs)
    zero_oacc()
    wait(wqb, sems.at[0])

    def layer1(g, c):
        q_proj(g, 0)
        issue_kv(v_hbm, vb, vsem, g)
        issue_w(wo_hbm, wob, osem.at[g], g * 48, 48, 4)
        wait(kb.at[pl.ds(g * GS, GS)], ksem.at[g])
        softmax(scores(g, 0), 0)

        @pl.when(g < NG - 1)
        def _():
            issue_kv(k_hbm, kb, ksem, g + 1)

        @pl.when(g == NG - 1)
        def _():
            issue_w(w1_hbm, w1b, sems.at[1], 0, 80, 4)
            issue_w(w2_hbm, w2b, sems.at[2], 0, 96, 4)

        wait(vb.at[pl.ds(g * GS, GS)], vsem.at[g])
        pv_mxu(g, 0, 0, 6)
        wait(wob.at[pl.ds(g * 48, 48)], osem.at[g])
        o_proj(g)
        return c

    lax.fori_loop(0, NG, layer1, 0)
    xs = add_attn(xs)
    xs = ffn(xs, lambda: wait(w1b, sems.at[1]), lambda: wait(w2b, sems.at[2]))

    layernorm_to_lhs(xs)
    zero_oacc()
    q_proj(0, 0)
    q_proj(1, 1)
    softmax(scores(0, 0), 0)

    def layer2(g, c):
        slot = g & 1
        ss = scores(g + 1, 1 - slot)
        q_proj(jnp.minimum(g + 2, NG - 1), slot)
        pv_vpu(g, slot, 0, 6)
        softmax(ss, 1 - slot)
        o_proj(g)
        return c

    lax.fori_loop(0, NG - 1, layer2, 0)
    pv_vpu(NG - 1, 1, DRAIN_MXU_U, 6)
    pv_mxu(NG - 1, 1, 0, DRAIN_MXU_U)
    o_proj(NG - 1)
    xs = add_attn(xs)
    xs = ffn(xs, lambda: None, lambda: None)
    out_ref[...] = jnp.concatenate([x[0:1, :] for x in xs], axis=1).astype(out_ref.dtype)


@jax.jit
def pallas_interleave_layers__sliding_block_cached__dense_activation_gelu__decode_kernel(
    A_x: jax.Array,
    A_k_cache: jax.Array,
    A_v_cache: jax.Array,
    A_wq: jax.Array,
    A_wo: jax.Array,
    B_x: jax.Array,
    B_w1: jax.Array,
    B_b1: jax.Array,
    B_w2: jax.Array,
    B_b2: jax.Array,
):
    del B_x
    cache = lambda a: _tile_order(jnp.transpose(a, (0, 1, 3, 2)).reshape(H * DH, SK), SK // 16)
    args = (
        A_x.reshape(1, D), cache(A_k_cache), cache(A_v_cache),
        _tile_order(A_wq, 384), _tile_order(A_wo, 80),
        _tile_order(B_w1, 96), B_b1.reshape(F // 128, 128),
        _tile_order(B_w2, 80), B_b2.reshape(D // 128, 128),
    )
    vm = pltpu.VMEM
    out = pl.pallas_call(
        _kernel,
        out_shape=jax.ShapeDtypeStruct((1, D), A_x.dtype),
        in_specs=[pl.BlockSpec(memory_space=pl.ANY)] * len(args),
        scratch_shapes=[
            vm((NS, WROWS, 128), BF16), vm((NS, WROWS, 128), BF16),
            vm((80, 384, 128), BF16), vm((384, 80, 128), BF16),
            vm((80, 96, 128), BF16), vm((96, 80, 128), BF16),
            vm((1, D), BF16), vm((F // 128, 128), BF16), vm((D // 128, 128), BF16),
            vm((10, 8, 128), F32), vm((2, 12, 8, 128), F32), vm((2, NJ, 8, 128), F32),
            vm((6, 8, 128), F32), vm((5, 8, 128), F32),
            pltpu.SemaphoreType.DMA((6,)), pltpu.SemaphoreType.DMA((NG,)),
            pltpu.SemaphoreType.DMA((NG,)), pltpu.SemaphoreType.DMA((NG,)),
        ],
        compiler_params=pltpu.CompilerParams(
            vmem_limit_bytes=122 * 2 ** 20, disable_bounds_checks=True),
        name="interleave_decode",
    )(*args)
    return out.reshape(1, 1, D)
```

```python
import jax
import jax.numpy as jnp
from jax import lax
import jax.experimental.pallas as pl
import jax.experimental.pallas.tpu as pltpu

D, F, H, DH, SK, W = 640, 1536, 32, 192, 32768, 4096
NS = H * DH // 8
HS = DH // 8
NP = H // 2
NJ = W // 256
WIN0 = (SK - W) // 16
WROWS = W // 16
SPLIT = 192
NB = 2
LAG_M, PER_M, LAG_V, PER_V = 20, 8, 150, 24
CM = 8.5
EPS = 1e-5
LOG2E = 1.4426950408889634
F32, BF16, I32 = jnp.float32, jnp.bfloat16, jnp.int32
NN = (((1,), (0,)), ((), ()))
NT = (((1,), (1,)), ((), ()))


def _tile_order(a, rows):
    r, c = a.shape
    a = a.reshape(r // 8, 8, c // 128, 128).transpose(0, 2, 1, 3)
    return a.reshape(-1, rows, 128)


def _rnd(x):
    return x.astype(BF16).astype(F32)


def _kernel(x_hbm, k_hbm, v_hbm, wq_hbm, wo_hbm, w1_hbm, b1_hbm, w2_hbm, b2_hbm,
            out_ref,
            kb, vb, wqb, wob, w1b, w2b, xb, b1b, b2b,
            xres, ylhs, qall, s0, s1, p0, p1, linv, zbuf, olhs, oacc, zeros, szero,
            sems, ksem, vsem, osem):
    kw, vw = kb.bitcast(I32), vb.bitcast(I32)
    wqw, wow = wqb.bitcast(I32), wob.bitcast(I32)
    w1w, w2w = w1b.bitcast(I32), w2b.bitcast(I32)

    sub = lax.broadcasted_iota(I32, (8, 128), 0)
    lane = lax.broadcasted_iota(I32, (8, 128), 1)

    def issue_kv(src, dst, sem, i):
        def body(t, c):
            s = i * (2 * HS) + 2 * t
            for r0, n, prio in ((0, SPLIT, 1), (SPLIT, WROWS - SPLIT, 0)):
                pltpu.make_async_copy(
                    src.at[pl.ds(s, 2), pl.ds(WIN0 + r0, n), :],
                    dst.at[pl.ds(s, 2), pl.ds(r0, n), :], sem.at[i]).start(priority=prio)
            return c
        lax.fori_loop(0, HS, body, 0)

    def issue_w(src, dst, sem, start, count, unit):
        big = unit * 3 // 4

        def body(t, c):
            s = start + unit * t
            for r0, n, prio in ((0, big, 1), (big, unit - big, 0)):
                pltpu.make_async_copy(src.at[pl.ds(s + r0, n)], dst.at[pl.ds(s + r0, n)],
                                      sem).start(priority=prio)
            return c
        lax.fori_loop(0, count // unit, body, 0)

    def issue_wq():
        def body(t, c):
            for r0, n, prio in ((0, 288, 1), (288, 96, 0)):
                pltpu.make_async_copy(wq_hbm.at[t, pl.ds(r0, n), :], wqb.at[t, pl.ds(r0, n), :],
                                      sems.at[0]).start(priority=prio)
            return c
        lax.fori_loop(0, 80, body, 0)

    def wait(ref, sem):
        pltpu.make_async_copy(ref, ref, sem).wait()

    def wait_kv(buf, sem, i):
        wait(buf.at[pl.ds(i * (2 * HS), 2 * HS)], sem.at[i])

    def wait_wo(i):
        wait(wob.at[pl.ds(i * HS, HS)], osem.at[i])

    def bcast_row(v, r):
        return jnp.broadcast_to(v[r:r + 1, :], (8, 128))

    def halves(v):
        rolled = pltpu.roll(v, 4, 0)
        return jnp.where(sub < 4, v, rolled), jnp.where(sub < 4, rolled, v)

    def all_rows_sum(v):
        return jnp.broadcast_to(jnp.sum(v, axis=0, keepdims=True), (8, 128))

    def gather(v, idx):
        return jnp.take_along_axis(v, idx, axis=1, mode="promise_in_bounds")

    same_c = ((lane >> 3) & 1) == (sub >> 2)

    def expand(v, half):
        return gather(v, 64 * half + ((lane >> 4) << 3) + (lane & 7))

    def down_lhs(v):
        return jnp.where(same_c, gather(v, (lane & ~8) + ((sub & 2) << 2)), 0.0)

    def layernorm_to_lhs(xs):
        tot = xs[0] + xs[1] + xs[2] + xs[3] + xs[4]
        mean = jnp.sum(tot, axis=1, keepdims=True) * (1.0 / D)
        ds = [x - mean for x in xs]
        sq = ds[0] * ds[0] + ds[1] * ds[1] + ds[2] * ds[2] + ds[3] * ds[3] + ds[4] * ds[4]
        var = jnp.sum(sq, axis=1, keepdims=True) * (1.0 / D)
        inv = 1.0 / jnp.sqrt(var + EPS)
        for t in range(10):
            ylhs[t] = jnp.where(same_c, _rnd(expand(ds[t // 2], t % 2) * inv), 0.0)

    def collect(outs):
        res = []
        for n in range(5):
            a, b = n, n + 5
            res.append(bcast_row(outs[a // 2], 4 * (a % 2)) + bcast_row(outs[b // 2], 4 * (b % 2) + 2))
        return res

    state = dict(me=0, clock=[0.0], toks=[[]], last=[0.0], never=None, turn=0)

    def publish(v):
        state["toks"][state["me"]].append((state["clock"][state["me"]], v))

    def tie(x, lag, period):
        me = state["me"]
        now = state["clock"][me]
        if len(state["toks"]) < 2 or now - state["last"][me] < period:
            return x
        old = [v for c, v in state["toks"][1 - me] if c <= now - lag]
        if not old:
            return x
        state["last"][me] = now
        state["turn"] += len(old[-1]) > 1
        tok = old[-1][state["turn"] % len(old[-1])]
        return jax.tree.map(lambda a: jnp.where(state["never"], pltpu.bitcast(tok, a.dtype), a), x)

    def weave(*streams):
        clock = [0.0] * len(streams)
        state.update(clock=clock, toks=[[] for _ in streams], last=[-1e9] * len(streams))
        if len(streams) > 1:
            state["never"] = zeros[...] != 0
        live = list(range(len(streams)))
        while live:
            i = min(live, key=lambda n: clock[n])
            state["me"] = i
            cost = next(streams[i], None)
            if cost is None:
                live.remove(i)
            else:
                clock[i] += cost

    def chain(*gens):
        for gen in gens:
            yield from gen

    def mm(a, words, dims=NN):
        rhs = pltpu.bitcast(words.reshape(64, 128), BF16)
        r = lax.dot_general(tie(a, LAG_M, PER_M), rhs, dims, preferred_element_type=F32)
        publish([r])
        return r

    def up_proj(ww, j, done):
        off = j * 8 if isinstance(j, int) else pl.multiple_of(j * 8, 8)
        acc = None
        for t in range(10):
            r = mm(ylhs[t], ww[8 * t:8 * t + 8, pl.ds(off, 8), :])
            acc = r if acc is None else acc + r
            yield CM
        done(acc)

    def down_proj(ww, u0, lhs):
        for t in range(5):
            acc = oacc[t]
            for n, a in enumerate(lhs):
                acc += mm(a(), ww[pl.ds(u0 + 8 * n, 8), 8 * t:8 * t + 8, :])
                yield CM
            oacc[t] = acc

    def q_proj(j):
        def done(q):
            for c, qc in enumerate(halves(_rnd(q))):
                for half in range(2):
                    qall[4 * j + 2 * c + half] = jnp.where(same_c, expand(qc, half), 0.0)
        return up_proj(wqw, j, done)

    def scores(h, sref):
        m = None
        for j in range(NJ):
            s = None
            for t in range(3):
                r = mm(qall[3 * h + t], kw[pl.ds(HS * h + 8 * t, 8), 8 * j:8 * j + 8, :])
                s = r if s is None else s + r
                yield CM
            s = s * (DH ** -0.5 * LOG2E)
            sref[j] = s
            m = s if m is None else jnp.maximum(m, s)
        sref[NJ] = jnp.maximum(m, pltpu.roll(m, 4, 0))

    def softmax(h, sref, pref):
        m = jnp.max(sref[NJ], axis=1, keepdims=True)
        l = None
        for j in range(NJ):
            e = jnp.exp2(sref[j] - m)
            pref[0, j] = e
            l = e if l is None else l + e
        l = l + pltpu.roll(l, 4, 0)
        linv[h] = jnp.broadcast_to(1.0 / jnp.sum(l, axis=1, keepdims=True), (8, 128))
        yield 0

    def pv_vpu(h, pref, z0):
        consts = (jnp.full((8, 128), 16, I32), jnp.full((8, 128), -65536, I32))
        shift, mask = consts
        for i in range(0, HS, NB):
            lo, hi = [None] * NB, [None] * NB
            ph = pref.at[szero[i // NB]]
            for j in range(NJ):
                p = ph[j]
                tied = tie(consts, LAG_V, PER_V)
                if tied is not consts:
                    shift, mask = tied
                for n in range(NB):
                    w = vw[HS * h + i + n, 8 * j:8 * j + 8, :]
                    a = pltpu.bitcast(w << shift, F32) * p
                    b = pltpu.bitcast(w & mask, F32) * p
                    lo[n] = a if j == 0 else lo[n] + a
                    hi[n] = b if j == 0 else hi[n] + b
                publish(lo + hi)
                yield 1.6 * NB
            for n in range(NB):
                zbuf[0, z0 + i + n] = lo[n]
                zbuf[1, z0 + i + n] = hi[n]

    def lanes_to_cols(strips):
        cols = {}
        place = (lane >> 1) - (sub & 3)
        for i in range(16):
            here = place == 4 * i
            for s in strips:
                if s % 16 == i:
                    v = jnp.where((lane & 1) == 0, jnp.sum(zbuf[0, s], axis=1, keepdims=True),
                                  jnp.sum(zbuf[1, s], axis=1, keepdims=True))
                    cols[s // 16] = jnp.where(here, v, cols.get(s // 16, 0.0))
        return cols

    def finish(h, outs):
        la, lb = linv[h], linv[h + 1]
        for u, inv in enumerate((la, jnp.where(lane < 64, la, lb), lb)):
            olhs[u] = down_lhs(_rnd(outs[u] * inv))

    def finish_vpu(h):
        cols = lanes_to_cols(range(2 * HS))
        finish(h, [all_rows_sum(cols[u]) for u in range(3)])
        yield 0

    def o_proj(i):
        return down_proj(wow, HS * i, [lambda u=u: olhs[u] for u in range(3)])

    def pv_mxu(h, pref, res):
        for t in range(3):
            acc = None
            for j in range(NJ):
                r = mm(_rnd(pref[0, j]), vw[pl.ds(HS * h + 8 * t, 8), 8 * j:8 * j + 8, :], NT)
                acc = r if acc is None else acc + r
                yield 1.25 * CM
            a = jnp.where(same_c, acc, 0.0)
            a = a + pltpu.roll(a, 4, 0)
            idx = ((lane & 56) << 1) + (lane & 7)
            res.append(gather(a, idx) + gather(a, idx + 8))

    def residual(bias=None):
        ys = collect([oacc[t] for t in range(5)])
        xs = [xres[n] + ys[n] for n in range(5)]
        if bias is not None:
            xs = [xs[n] + bcast_row(bias, n) for n in range(5)]
        for n in range(5):
            xres[n] = xs[n]
            oacc[n] = jnp.zeros((8, 128), F32)
        return xs

    small = [pltpu.make_async_copy(s, d, sems.at[3 + i])
             for i, (s, d) in enumerate(((x_hbm, xb), (b1_hbm, b1b), (b2_hbm, b2b)))]
    for c in small:
        c.start()
    issue_wq()
    issue_kv(k_hbm, kb, ksem, 0)
    issue_w(wo_hbm, wob, osem.at[0], 0, HS, 4)
    zeros[...] = jnp.zeros((8, 128), I32)
    for n in range(HS // NB):
        szero[n] = 0
    for c in small:
        c.wait()
    x0 = xb[...].astype(F32)
    for n in range(5):
        xres[n] = jnp.broadcast_to(x0[:, 128 * n:128 * n + 128], (8, 128))
        oacc[n] = jnp.zeros((8, 128), F32)
    zbuf[...] = jnp.zeros(zbuf.shape, F32)
    issue_kv(k_hbm, kb, ksem, 1)
    issue_kv(v_hbm, vb, vsem, 0)
    wait(wqb, sems.at[0])
    wait_kv(kb, ksem, 0)
    wait_wo(0)

    def layer(li, carry):
        first = li == 0
        layernorm_to_lhs([xres[n] for n in range(5)])
        weave(chain(q_proj(0), q_proj(1), scores(0, s0), q_proj(2), softmax(0, s0, p0),
                    scores(1, s1)))
        linv[1] = jnp.zeros((8, 128), F32)

        def step(i, c):
            @pl.when(first)
            def _():
                @pl.when(i < NP - 2)
                def _():
                    issue_kv(k_hbm, kb, ksem, i + 2)
                issue_w(wo_hbm, wob, osem.at[i + 1], (i + 1) * HS, HS, 4)
                issue_kv(v_hbm, vb, vsem, i + 1)

                @pl.when(i == NP - 2)
                def _():
                    issue_w(w1_hbm, w1b, sems.at[1], 0, 80, 4)
                wait_kv(kb, ksem, i + 1)
                wait_kv(vb, vsem, i)
                wait_wo(i + 1)

            h = 2 * i
            prev = jnp.maximum(i - 1, 0)
            weave(chain(scores(h + 2, s0), scores(h + 3, s1), o_proj(prev),
                        q_proj(jnp.minimum(h + 3, 22)),
                        q_proj(jnp.minimum(h + 4, 23))),
                  chain(finish_vpu(2 * prev), softmax(h + 1, s1, p1), pv_vpu(h, p0, 0),
                        softmax(h + 2, s0, p0), pv_vpu(h + 1, p1, HS)))
            return c

        lax.fori_loop(0, NP - 1, step, 0)

        @pl.when(first)
        def _():
            issue_w(w2_hbm, w2b, sems.at[2], 0, 96, 4)
            wait_kv(vb, vsem, NP - 1)

        last = []
        weave(chain(softmax(H - 1, s1, p1), finish_vpu(H - 4),
                    pv_mxu(H - 1, p1, last), o_proj(NP - 2)),
              pv_vpu(H - 2, p0, 0))
        cols = lanes_to_cols(range(HS))
        finish(H - 2, [all_rows_sum(cols[0]),
                       jnp.where(lane < 64, all_rows_sum(cols[1]), last[0]),
                       jnp.where(lane < 64, last[1], last[2])])
        weave(o_proj(NP - 1))
        layernorm_to_lhs(residual())
        zbuf[...] = jnp.zeros(zbuf.shape, F32)

        @pl.when(first)
        def _():
            wait(w1b, sems.at[1])

        b1 = b1b[...].astype(F32)

        def hidden(j):
            def done(hid):
                bias = jnp.where(sub < 4, bcast_row(b1, 2 * j), bcast_row(b1, 2 * j + 1))
                act = _rnd(jax.nn.gelu(hid + bias, approximate=True))
                for c, v in enumerate(halves(act)):
                    qall[2 * j + c] = down_lhs(v)
            return up_proj(w1w, j, done)

        weave(chain(*[hidden(j) for j in range(6)]))

        @pl.when(first)
        def _():
            wait(w2b, sems.at[2])

        weave(down_proj(w2w, 0, [lambda u=u: qall[u] for u in range(12)]))
        residual(b2b[...].astype(F32))
        return carry

    lax.fori_loop(0, 2, layer, 0)
    out_ref[...] = jnp.concatenate([xres[n, 0:1, :] for n in range(5)], axis=1).astype(out_ref.dtype)


@jax.jit
def pallas_interleave_layers__sliding_block_cached__dense_activation_gelu__decode_kernel(
    A_x: jax.Array,
    A_k_cache: jax.Array,
    A_v_cache: jax.Array,
    A_wq: jax.Array,
    A_wo: jax.Array,
    B_x: jax.Array,
    B_w1: jax.Array,
    B_b1: jax.Array,
    B_w2: jax.Array,
    B_b2: jax.Array,
):
    del B_x
    cache = lambda a: _tile_order(jnp.transpose(a, (0, 1, 3, 2)).reshape(H * DH, SK), SK // 16)
    args = (
        A_x.reshape(1, D), cache(A_k_cache), cache(A_v_cache),
        _tile_order(A_wq, 384), _tile_order(A_wo, 80),
        _tile_order(B_w1, 96), B_b1.reshape(F // 128, 128),
        _tile_order(B_w2, 80), B_b2.reshape(D // 128, 128),
    )
    vm = pltpu.VMEM
    vregs = lambda *n: vm((*n, 8, 128), F32)
    out = pl.pallas_call(
        _kernel,
        out_shape=jax.ShapeDtypeStruct((1, D), A_x.dtype),
        in_specs=[pl.BlockSpec(memory_space=pl.ANY)] * len(args),
        scratch_shapes=[
            vm((NS, WROWS, 128), BF16), vm((NS, WROWS, 128), BF16),
            vm((80, 384, 128), BF16), vm((384, 80, 128), BF16),
            vm((80, 96, 128), BF16), vm((96, 80, 128), BF16),
            vm((1, D), BF16), vm((F // 128, 128), BF16), vm((D // 128, 128), BF16),
            vregs(5), vregs(10), vregs(3 * H), vregs(NJ + 1), vregs(NJ + 1),
            vregs(1, NJ), vregs(1, NJ), vregs(H), vregs(2, 2 * HS), vregs(3), vregs(5),
            vm((8, 128), I32), pltpu.SMEM((HS // NB,), I32),
            pltpu.SemaphoreType.DMA((6,)), pltpu.SemaphoreType.DMA((NP,)),
            pltpu.SemaphoreType.DMA((NP,)), pltpu.SemaphoreType.DMA((NP,)),
        ],
        compiler_params=pltpu.CompilerParams(
            vmem_limit_bytes=122 * 2 ** 20, disable_bounds_checks=True),
        name="interleave_decode",
    )(*args)
    return out.reshape(1, 1, D)
```

```python
import jax
import jax.numpy as jnp
from jax import lax
import jax.experimental.pallas as pl
import jax.experimental.pallas.tpu as pltpu

D, F, H, DH, SK, W = 640, 1536, 32, 192, 32768, 4096
NS = H * DH // 8
HS = DH // 8
NP = H // 2
NJ = W // 256
WIN0 = (SK - W) // 16
WROWS = W // 16
K0, V0, WO0, WQ0, SLOT = 0, 2 * HS, 4 * HS, 4 * HS + 8, 4 * HS + 16
SPLIT = 192
NB = 2
LAG_M, PER_M, LAG_V, PER_V = 20, 16, 150, 24
CM = 8.5
EPS = 1e-5
LOG2E = 1.4426950408889634
F32, BF16, I32 = jnp.float32, jnp.bfloat16, jnp.int32
NN = (((1,), (0,)), ((), ()))
NT = (((1,), (1,)), ((), ()))


def _tile_order(a, rows):
    r, c = a.shape
    a = a.reshape(r // 8, 8, c // 128, 128).transpose(0, 2, 1, 3)
    return a.reshape(-1, rows, 128)


def _rnd(x):
    return x.astype(BF16).astype(F32)


def _kernel(x_hbm, k_hbm, v_hbm, wq_hbm, wo_hbm, w1_hbm, b1_hbm, w2_hbm, b2_hbm,
            out_ref,
            big, w1b, w2b, xb, b1b, b2b,
            xres, ylhs, hlhs, q0, q1, s0, s1, p0, p1, linv, zbuf, olhs, oacc, zeros,
            sems, ksem, vsem, osem):
    bigw = big.bitcast(I32)
    w1w, w2w = w1b.bitcast(I32), w2b.bitcast(I32)

    sub = lax.broadcasted_iota(I32, (8, 128), 0)
    lane = lax.broadcasted_iota(I32, (8, 128), 1)

    def issue_strips(src, src0, row0, dst0, count, sem):
        def body(t, c):
            for r0, n, prio in ((0, SPLIT, 1), (SPLIT, WROWS - SPLIT, 0)):
                pltpu.make_async_copy(
                    src.at[pl.ds(src0 + 2 * t, 2), pl.ds(row0 + r0, n), :],
                    big.at[pl.ds(dst0 + 2 * t, 2), pl.ds(r0, n), :], sem).start(priority=prio)
            return c
        lax.fori_loop(0, count // 2, body, 0)

    def issue_k(i):
        issue_strips(k_hbm, 2 * HS * i, WIN0, SLOT * i + K0, 2 * HS, ksem.at[i])

    def issue_v(i):
        issue_strips(v_hbm, 2 * HS * i, WIN0, SLOT * i + V0, 2 * HS, vsem.at[i])

    def issue_wo(i):
        pair = (i + NP - 1) % NP

        def body(t, c):
            for r0, n, prio in ((0, 176, 1), (176, 64, 0)):
                pltpu.make_async_copy(wo_hbm.at[8 * pair + t, pl.ds(r0, n), :],
                                      big.at[SLOT * i + WO0 + t, pl.ds(r0, n), :],
                                      osem.at[i]).start(priority=prio)
            return c
        lax.fori_loop(0, 8, body, 0)

    def issue_w(src, dst, sem, start, count, unit):
        most = unit * 3 // 4

        def body(t, c):
            s = start + unit * t
            for r0, n, prio in ((0, most, 1), (most, unit - most, 0)):
                pltpu.make_async_copy(src.at[pl.ds(s + r0, n)], dst.at[pl.ds(s + r0, n)],
                                      sem).start(priority=prio)
            return c
        lax.fori_loop(0, count // unit, body, 0)

    def wait(ref, sem):
        pltpu.make_async_copy(ref, ref, sem).wait()

    def wait_k(i):
        wait(big.at[pl.ds(SLOT * i + K0, 2 * HS)], ksem.at[i])

    def wait_v(i):
        wait(big.at[pl.ds(SLOT * i + V0, 2 * HS)], vsem.at[i])

    def wait_wo(i):
        wait(big.at[pl.ds(SLOT * i + WO0, 8), pl.ds(0, 240), :], osem.at[i])

    def unpair_wq(half):
        def body(u, c):
            src = bigw.at[pl.ds(SLOT * (NP - 2 + half) + 3 * u, 3)]
            for j in range(24):
                a = src[j // 16, pl.ds(8 * (j % 16), 8), :]
                b = src[(24 + j) // 16, pl.ds(8 * ((24 + j) % 16), 8), :]
                both = (jnp.where(sub < 4, a, pltpu.roll(b, 4, 0)),
                        jnp.where(sub < 4, pltpu.roll(a, 4, 0), b))
                for cb, w in zip((2 * j, 2 * j + 1), both):
                    n = 40 * (cb % 3) + 20 * half + u
                    bigw[SLOT * ((cb // 3 + NP - 2) % NP) + WQ0 + (n >> 4),
                         pl.ds(pl.multiple_of(8 * (n & 15), 8), 8), :] = w
            return c
        lax.fori_loop(0, 20, body, 0)

    def bcast_row(v, r):
        return jnp.broadcast_to(v[r:r + 1, :], (8, 128))

    def halves(v):
        rolled = pltpu.roll(v, 4, 0)
        return jnp.where(sub < 4, v, rolled), jnp.where(sub < 4, rolled, v)

    def all_rows_sum(v):
        return jnp.broadcast_to(jnp.sum(v, axis=0, keepdims=True), (8, 128))

    def gather(v, idx):
        return jnp.take_along_axis(v, idx, axis=1, mode="promise_in_bounds")

    same_c = ((lane >> 3) & 1) == (sub >> 2)

    def expand(v, half):
        return gather(v, 64 * half + ((lane >> 4) << 3) + (lane & 7))

    def down_lhs(v):
        return jnp.where(same_c, gather(v, (lane & ~8) + ((sub & 2) << 2)), 0.0)

    def layernorm(xs):
        tot = xs[0] + xs[1] + xs[2] + xs[3] + xs[4]
        mean = jnp.sum(tot, axis=1, keepdims=True) * (1.0 / D)
        ds = [x - mean for x in xs]
        sq = ds[0] * ds[0] + ds[1] * ds[1] + ds[2] * ds[2] + ds[3] * ds[3] + ds[4] * ds[4]
        var = jnp.sum(sq, axis=1, keepdims=True) * (1.0 / D)
        inv = 1.0 / jnp.sqrt(var + EPS)
        return ds, inv

    def collect(outs):
        res = []
        for n in range(5):
            a, b = n, n + 5
            res.append(bcast_row(outs[a // 2], 4 * (a % 2)) + bcast_row(outs[b // 2], 4 * (b % 2) + 2))
        return res

    state = dict(me=0, clock=[0.0], toks=[[]], last=[0.0], never=None, turn=0)

    def publish(v):
        state["toks"][state["me"]].append((state["clock"][state["me"]], v))

    def tie(x, lag, period):
        me = state["me"]
        now = state["clock"][me]
        if len(state["toks"]) < 2 or now - state["last"][me] < period:
            return x
        old = [v for c, v in state["toks"][1 - me] if c <= now - lag]
        if not old:
            return x
        state["last"][me] = now
        state["turn"] += len(old[-1]) > 1
        tok = sum(old[-1][1:], old[-1][0])
        return jax.tree.map(lambda a: jnp.where(state["never"], pltpu.bitcast(tok, a.dtype), a), x)

    def weave(*streams):
        clock = [0.0] * len(streams)
        state.update(clock=clock, toks=[[] for _ in streams], last=[-1e9] * len(streams))
        if len(streams) > 1:
            state["never"] = zeros[...] != 0
        live = list(range(len(streams)))
        while live:
            i = min(live, key=lambda n: clock[n])
            state["me"] = i
            cost = next(streams[i], None)
            if cost is None:
                live.remove(i)
            else:
                clock[i] += cost

    def chain(*gens):
        for gen in gens:
            yield from gen

    def mm(a, words, dims=NN):
        rhs = pltpu.bitcast(words.reshape(64, 128), BF16)
        r = lax.dot_general(tie(a, LAG_M, PER_M), rhs, dims, preferred_element_type=F32)
        publish([r])
        return r

    def up_proj(ww, j, done):
        acc = None
        for t in range(10):
            r = mm(ylhs[t], ww[8 * t:8 * t + 8, 8 * j:8 * j + 8, :])
            acc = r if acc is None else acc + r
            yield CM
        done(acc)

    def down_proj(lhs, count, tile):
        for t in range(5):
            acc = oacc[t]
            for n in range(count):
                acc += mm(lhs[n], tile(n, t))
                yield CM
            oacc[t] = acc

    def o_proj(slot):
        def tile(n, t):
            return jnp.concatenate(
                [slot[WO0 + u // 3, pl.ds(40 * (u % 3) + 8 * t, 8), :]
                 for u in range(8 * n, 8 * n + 8)], axis=0)
        return down_proj(olhs, 3, tile)

    def q_proj(slot, dst):
        for cb in range(3):
            q = None
            for t in range(5):
                n = 5 * cb + t
                r = mm(ylhs[t], slot[WQ0 + n // 2, pl.ds(64 * (n % 2), 64), :])
                q = r if q is None else q + r
                yield CM
            q = _rnd(q)
            for half in range(2):
                dst[2 * cb + half] = jnp.where(same_c, expand(q, half), 0.0)

    def scores(q, h, kv, s_0, sref):
        m = None
        for j in range(NJ):
            s = None
            for t in range(3):
                r = mm(q[3 * h + t], kv[pl.ds(s_0 + 8 * t, 8), 8 * j:8 * j + 8, :])
                s = r if s is None else s + r
                yield CM
            s = s * (DH ** -0.5 * LOG2E)
            sref[j] = s
            m = s if m is None else jnp.maximum(m, s)
        sref[NJ] = jnp.maximum(m, pltpu.roll(m, 4, 0))

    def softmax(h, sref, pref):
        m = jnp.max(sref[NJ], axis=1, keepdims=True)
        l = None
        for j in range(NJ):
            e = jnp.exp2(sref[j] - m)
            pref[j] = e
            l = e if l is None else l + e
        l = l + pltpu.roll(l, 4, 0)
        linv[h] = jnp.broadcast_to(1.0 / jnp.sum(l, axis=1, keepdims=True), (8, 128))
        yield 0

    def pv_vpu(kv, s_0, pref, z0):
        consts = (jnp.full((8, 128), 16, I32), jnp.full((8, 128), -65536, I32))
        shift, mask = consts
        for i in range(0, HS, NB):
            lo, hi = [None] * NB, [None] * NB
            for j in range(NJ):
                p = pref[j]
                tied = tie(consts, LAG_V, PER_V)
                if tied is not consts:
                    shift, mask = tied
                for n in range(NB):
                    w = kv[s_0 + i + n, 8 * j:8 * j + 8, :]
                    a = pltpu.bitcast(w << shift, F32) * p
                    b = pltpu.bitcast(w & mask, F32) * p
                    lo[n] = a if j == 0 else lo[n] + a
                    hi[n] = b if j == 0 else hi[n] + b
                publish(lo + hi)
                yield 1.6 * NB
            for n in range(NB):
                zbuf[0, z0 + i + n] = lo[n]
                zbuf[1, z0 + i + n] = hi[n]

    def lanes_to_cols(strips):
        cols = {}
        place = (lane >> 1) - (sub & 3)
        for i in range(16):
            here = place == 4 * i
            for s in strips:
                if s % 16 == i:
                    v = jnp.where((lane & 1) == 0, jnp.sum(zbuf[0, s], axis=1, keepdims=True),
                                  jnp.sum(zbuf[1, s], axis=1, keepdims=True))
                    cols[s // 16] = jnp.where(here, v, cols.get(s // 16, 0.0))
        return cols

    def finish(h, outs):
        la, lb = linv[h], linv[h + 1]
        for u, inv in enumerate((la, jnp.where(lane < 64, la, lb), lb)):
            olhs[u] = down_lhs(_rnd(outs[u] * inv))

    def finish_vpu(h):
        cols = lanes_to_cols(range(2 * HS))
        finish(h, [all_rows_sum(cols[u]) for u in range(3)])
        yield 0

    def pv_mxu(s_0, pref, res):
        for t in range(3):
            acc = None
            for j in range(NJ):
                r = mm(_rnd(pref[j]), bigw[pl.ds(s_0 + 8 * t, 8), 8 * j:8 * j + 8, :], NT)
                acc = r if acc is None else acc + r
                yield 1.25 * CM
            a = jnp.where(same_c, acc, 0.0)
            a = a + pltpu.roll(a, 4, 0)
            idx = ((lane & 56) << 1) + (lane & 7)
            res.append(gather(a, idx) + gather(a, idx + 8))

    def residual(bias=None):
        ys = collect([oacc[t] for t in range(5)])
        xs = [xres[n] + ys[n] for n in range(5)]
        if bias is not None:
            xs = [xs[n] + bcast_row(bias, n) for n in range(5)]
        for n in range(5):
            xres[n] = xs[n]
            oacc[n] = jnp.zeros((8, 128), F32)
        return xs

    small = [pltpu.make_async_copy(s, d, sems.at[3 + i])
             for i, (s, d) in enumerate(((x_hbm, xb), (b1_hbm, b1b), (b2_hbm, b2b)))]
    for c in small:
        c.start()
    for half in range(2):
        issue_strips(wq_hbm, 60 * half, 0, SLOT * (NP - 2 + half), 60, sems.at[6 + half])
    zeros[...] = jnp.zeros((8, 128), I32)
    for c in small:
        c.wait()
    x0 = xb[...].astype(F32)
    for n in range(5):
        xres[n] = jnp.broadcast_to(x0[:, 128 * n:128 * n + 128], (8, 128))
        oacc[n] = jnp.zeros((8, 128), F32)
    zbuf[...] = jnp.zeros(zbuf.shape, F32)
    for half in range(2):
        issue_k(half)
        wait(big.at[pl.ds(SLOT * (NP - 2 + half), 60)], sems.at[6 + half])
        unpair_wq(half)
    issue_wo(0)
    issue_v(0)
    wait_k(0)

    def slot_at(i):
        return bigw.at[pl.ds(SLOT * i, SLOT)]

    def layer(li, carry):
        first = li == 0
        ds, inv = layernorm([xres[n] for n in range(5)])
        for t in range(5):
            ylhs[t] = _rnd(ds[t] * inv)
        weave(chain(q_proj(slot_at(NP - 2), q0), q_proj(slot_at(NP - 1), q1),
                    scores(q0, 0, bigw, K0, s0), softmax(0, s0, p0),
                    scores(q0, 1, bigw, K0 + HS, s1)))
        linv[1] = jnp.zeros((8, 128), F32)

        def step(i, c):
            @pl.when(first)
            def _():
                @pl.when(i < NP - 2)
                def _():
                    issue_k(i + 2)
                issue_wo(i + 1)
                issue_v(i + 1)

                @pl.when(i == NP - 2)
                def _():
                    issue_w(w1_hbm, w1b, sems.at[1], 0, 80, 4)
                wait_k(i + 1)
                wait_wo(i)
                wait_v(i)

            h = 2 * i
            kv = bigw.at[pl.ds(SLOT * i, SLOT + 2 * HS)]
            prev = jnp.maximum(h - 2, 0)
            weave(chain(scores(q1, 0, kv, SLOT, s0), scores(q1, 1, kv, SLOT + HS, s1),
                        q_proj(kv, q1), o_proj(kv)),
                  chain(finish_vpu(prev), softmax(h + 1, s1, p1), pv_vpu(kv, V0, p0, 0),
                        softmax(h + 2, s0, p0), pv_vpu(kv, V0 + HS, p1, HS)))
            return c

        lax.fori_loop(0, NP - 1, step, 0)

        @pl.when(first)
        def _():
            issue_w(w2_hbm, w2b, sems.at[2], 0, 96, 4)
            wait_wo(NP - 1)
            wait_v(NP - 1)

        last = []
        v_last = SLOT * (NP - 1) + V0
        weave(chain(softmax(H - 1, s1, p1), finish_vpu(H - 4),
                    o_proj(slot_at(NP - 1)), pv_mxu(v_last + HS, p1, last)),
              pv_vpu(bigw, v_last, p0, 0))
        cols = lanes_to_cols(range(HS))
        finish(H - 2, [all_rows_sum(cols[0]),
                       jnp.where(lane < 64, all_rows_sum(cols[1]), last[0]),
                       jnp.where(lane < 64, last[1], last[2])])
        weave(o_proj(slot_at(0)))
        ds, inv = layernorm(residual())
        for t in range(10):
            ylhs[t] = jnp.where(same_c, _rnd(expand(ds[t // 2], t % 2) * inv), 0.0)
        zbuf[...] = jnp.zeros(zbuf.shape, F32)

        @pl.when(first)
        def _():
            wait(w1b, sems.at[1])

        b1 = b1b[...].astype(F32)

        def hidden(j):
            def done(hid):
                bias = jnp.where(sub < 4, bcast_row(b1, 2 * j), bcast_row(b1, 2 * j + 1))
                act = _rnd(jax.nn.gelu(hid + bias, approximate=True))
                for c, v in enumerate(halves(act)):
                    hlhs[2 * j + c] = down_lhs(v)
            return up_proj(w1w, j, done)

        weave(chain(*[hidden(j) for j in range(6)]))

        @pl.when(first)
        def _():
            wait(w2b, sems.at[2])

        weave(down_proj(hlhs, 12, lambda n, t: w2w[8 * n:8 * n + 8, 8 * t:8 * t + 8, :]))
        residual(b2b[...].astype(F32))
        return carry

    lax.fori_loop(0, 2, layer, 0)
    out_ref[...] = jnp.concatenate([xres[n, 0:1, :] for n in range(5)], axis=1).astype(out_ref.dtype)


@jax.jit
def pallas_interleave_layers__sliding_block_cached__dense_activation_gelu__decode_kernel(
    A_x: jax.Array,
    A_k_cache: jax.Array,
    A_v_cache: jax.Array,
    A_wq: jax.Array,
    A_wo: jax.Array,
    B_x: jax.Array,
    B_w1: jax.Array,
    B_b1: jax.Array,
    B_w2: jax.Array,
    B_b2: jax.Array,
):
    del B_x
    cache = lambda a: _tile_order(jnp.transpose(a, (0, 1, 3, 2)).reshape(H * DH, SK), SK // 16)
    args = (
        A_x.reshape(1, D), cache(A_k_cache), cache(A_v_cache),
        _tile_order(A_wq, 256), _tile_order(A_wo, 240),
        _tile_order(B_w1, 96), B_b1.reshape(F // 128, 128),
        _tile_order(B_w2, 80), B_b2.reshape(D // 128, 128),
    )
    vm = pltpu.VMEM
    vregs = lambda *n: vm((*n, 8, 128), F32)
    out = pl.pallas_call(
        _kernel,
        out_shape=jax.ShapeDtypeStruct((1, D), A_x.dtype),
        in_specs=[pl.BlockSpec(memory_space=pl.ANY)] * len(args),
        scratch_shapes=[
            vm((NP * SLOT, WROWS, 128), BF16),
            vm((80, 96, 128), BF16), vm((96, 80, 128), BF16),
            vm((1, D), BF16), vm((F // 128, 128), BF16), vm((D // 128, 128), BF16),
            vregs(5), vregs(10), vregs(12), vregs(6), vregs(6), vregs(NJ + 1), vregs(NJ + 1),
            vregs(NJ), vregs(NJ), vregs(H), vregs(2, 2 * HS), vregs(3), vregs(5),
            vm((8, 128), I32),
            pltpu.SemaphoreType.DMA((8,)), pltpu.SemaphoreType.DMA((NP,)),
            pltpu.SemaphoreType.DMA((NP,)), pltpu.SemaphoreType.DMA((NP,)),
        ],
        compiler_params=pltpu.CompilerParams(
            vmem_limit_bytes=122 * 2 ** 20, disable_bounds_checks=True),
        name="interleave_decode",
    )(*args)
    return out.reshape(1, 1, D)
```

```python
import jax
import jax.numpy as jnp
from jax import lax
import jax.experimental.pallas as pl
import jax.experimental.pallas.tpu as pltpu

D, F, H, DH, SK, W = 640, 1536, 32, 192, 32768, 4096
NS = H * DH // 8
HS = DH // 8
NP = H // 2
NJ = W // 256
WIN0 = (SK - W) // 16
WROWS = W // 16
WIDE = [(s, j) for s in range(32) for j in (3, 7, 11, 15)]
K0, V0, WO0, WQ0, LO0 = 0, 2 * HS, 4 * HS, 4 * HS + 8, 4 * HS + 16
SLOT = LO0 + len(WIDE) // 16
SPLIT = 64
LAG_M, PER_M, LAG_V, PER_V = 20, 16, 150, 24
CM = 8.0
EPS = 1e-5
LOG2E = 1.4426950408889634
F32, BF16, I32 = jnp.float32, jnp.bfloat16, jnp.int32
NN = (((1,), (0,)), ((), ()))
NT = (((1,), (1,)), ((), ()))


def _tile_order(a, rows):
    r, c = a.shape
    a = a.reshape(r // 8, 8, c // 128, 128).transpose(0, 2, 1, 3)
    return a.reshape(-1, rows, 128)


def _rnd(x):
    return x.astype(BF16).astype(F32)


def _kernel(x_hbm, k_hbm, v_hbm, wq_hbm, wo_hbm, w1_hbm, b1_hbm, w2_hbm, b2_hbm,
            out_ref,
            big, w1b, w2b, xb, b1b, b2b,
            xres, ylhs, hlhs, q0, q1, s0, s1, p0, p1, linv, zbuf, olhs, oacc, zeros,
            sems):
    bigw = big.bitcast(I32)
    w1w, w2w = w1b.bitcast(I32), w2b.bitcast(I32)

    sub = lax.broadcasted_iota(I32, (8, 128), 0)
    lane = lax.broadcasted_iota(I32, (8, 128), 1)

    def copy(src, row0, dst, sem):
        rows = dst.shape[-2]
        for r0, n, prio in ((0, rows - SPLIT, 1), (rows - SPLIT, SPLIT, 0)):
            pltpu.make_async_copy(src.at[:, pl.ds(row0 + r0, n), :], dst.at[:, pl.ds(r0, n), :],
                                  sem).start(priority=prio)

    def issue_weight(src, src0, dst, dst0, count, sem):
        def body(t, c):
            s = jnp.where(t < count - 1, (8 * t) % (count - 1), t)
            copy(src.at[pl.ds(src0 + s, 1)], 0, dst.at[pl.ds(dst0 + s, 1)], sem)
            return c
        lax.fori_loop(0, count, body, 0)

    def issue_k(i, sem):
        def body(t, c):
            copy(k_hbm.at[pl.ds(2 * HS * i + 2 * t, 2)], WIN0,
                 big.at[pl.ds(SLOT * i + K0 + 2 * t, 2)], sem)
            return c
        lax.fori_loop(0, HS, body, 0)

    def issue_v_wo(i, sem):
        def body(t, c):
            copy(wo_hbm.at[pl.ds(8 * ((i + NP - 1) % NP) + t, 1)], 0,
                 big.at[pl.ds(SLOT * i + WO0 + t, 1), pl.ds(0, 240), :], sem)
            for n in range(0, 6, 2):
                copy(v_hbm.at[pl.ds(2 * HS * i + 6 * t + n, 2)], WIN0,
                     big.at[pl.ds(SLOT * i + V0 + 6 * t + n, 2)], sem)
            return c
        lax.fori_loop(0, 8, body, 0)

    def wait(ref, sem):
        pltpu.make_async_copy(ref, ref, sem).wait()

    def wait_k(i, sem):
        wait(big.at[pl.ds(SLOT * i + K0, 2 * HS)], sem)

    def wait_v_wo(i, sem):
        wait(big.at[pl.ds(SLOT * i + V0, 2 * HS)], sem)
        wait(big.at[pl.ds(SLOT * i + WO0, 8), pl.ds(0, 240), :], sem)

    def widen_v(i, strips=2 * HS):
        slot = bigw.at[pl.ds(SLOT * i, SLOT)]
        for n, (s, j) in enumerate(WIDE):
            if s < strips:
                w = slot[V0 + s, 8 * j:8 * j + 8, :]
                slot[LO0 + n // 16, pl.ds(8 * (n % 16), 8), :] = w << 16
                slot[V0 + s, 8 * j:8 * j + 8, :] = w & -65536

    def unpair_wq(half):
        def body(u, c):
            src = bigw.at[pl.ds(SLOT * (NP - 2 + half) + 3 * u, 3)]
            for j in range(24):
                a = src[j // 16, pl.ds(8 * (j % 16), 8), :]
                b = src[(24 + j) // 16, pl.ds(8 * ((24 + j) % 16), 8), :]
                both = (jnp.where(sub < 4, a, pltpu.roll(b, 4, 0)),
                        jnp.where(sub < 4, pltpu.roll(a, 4, 0), b))
                for cb, w in zip((2 * j, 2 * j + 1), both):
                    n = 40 * (cb % 3) + 20 * half + u
                    bigw[SLOT * ((cb // 3 + NP - 2) % NP) + WQ0 + (n >> 4),
                         pl.ds(pl.multiple_of(8 * (n & 15), 8), 8), :] = w
            return c
        lax.fori_loop(0, 20, body, 0)

    def bcast_row(v, r):
        return jnp.broadcast_to(v[r:r + 1, :], (8, 128))

    def halves(v):
        rolled = pltpu.roll(v, 4, 0)
        return jnp.where(sub < 4, v, rolled), jnp.where(sub < 4, rolled, v)

    def all_rows_sum(v):
        return jnp.broadcast_to(jnp.sum(v, axis=0, keepdims=True), (8, 128))

    def gather(v, idx):
        return jnp.take_along_axis(v, idx, axis=1, mode="promise_in_bounds")

    same_c = ((lane >> 3) & 1) == (sub >> 2)

    def expand(v, half):
        return gather(v, 64 * half + ((lane >> 4) << 3) + (lane & 7))

    def down_lhs(v):
        return jnp.where(same_c, gather(v, (lane & ~8) + ((sub & 2) << 2)), 0.0)

    def layernorm(xs):
        tot = xs[0] + xs[1] + xs[2] + xs[3] + xs[4]
        mean = jnp.sum(tot, axis=1, keepdims=True) * (1.0 / D)
        ds = [x - mean for x in xs]
        sq = ds[0] * ds[0] + ds[1] * ds[1] + ds[2] * ds[2] + ds[3] * ds[3] + ds[4] * ds[4]
        var = jnp.sum(sq, axis=1, keepdims=True) * (1.0 / D)
        inv = 1.0 / jnp.sqrt(var + EPS)
        return ds, inv

    def collect(outs):
        res = []
        for n in range(5):
            a, b = n, n + 5
            res.append(bcast_row(outs[a // 2], 4 * (a % 2)) + bcast_row(outs[b // 2], 4 * (b % 2) + 2))
        return res

    state = dict(me=0, clock=[0.0], toks=[[]], last=[0.0], never=None)

    def publish(v):
        state["toks"][state["me"]].append((state["clock"][state["me"]], v))

    def tie(x, lag, period):
        me = state["me"]
        now = state["clock"][me]
        if len(state["toks"]) < 2 or now - state["last"][me] < period:
            return x
        old = [v for c, v in state["toks"][1 - me] if c <= now - lag]
        if not old:
            return x
        state["last"][me] = now
        tok = sum(old[-1][1:], old[-1][0])
        return jax.tree.map(lambda a: jnp.where(state["never"], pltpu.bitcast(tok, a.dtype), a), x)

    def weave(*streams, tied=True):
        clock = [0.0] * len(streams)
        state.update(clock=clock, toks=[[] for _ in streams], last=[-1e9 if tied else 1e9] * len(streams))
        if len(streams) > 1:
            state["never"] = zeros[...] != 0
        live = list(range(len(streams)))
        while live:
            i = min(live, key=lambda n: clock[n])
            state["me"] = i
            cost = next(streams[i], None)
            if cost is None:
                live.remove(i)
            else:
                clock[i] += cost

    def chain(*gens):
        for gen in gens:
            yield from gen

    def mm(a, words, dims=NN):
        rhs = pltpu.bitcast(words.reshape(64, 128), BF16)
        r = lax.dot_general(tie(a, LAG_M, PER_M), rhs, dims, preferred_element_type=F32)
        publish([r])
        return r

    def vregs_of(ref, ns, per=16):
        return jnp.concatenate([ref[n // per, pl.ds(8 * (n % per), 8), :] for n in ns], axis=0)

    def down_proj(lhs, count, ref, n0, per):
        acc = [oacc[t] for t in range(5)]
        for n in range(count):
            for t in range(5):
                acc[t] += mm(lhs[n], vregs_of(
                    ref, [n0 + 5 * u + t for u in range(8 * n, 8 * n + 8)], per))
                yield CM
        for t in range(5):
            oacc[t] = acc[t]

    def o_proj(slot):
        return down_proj(olhs, 3, slot, 15 * WO0, 15)

    def q_proj(slot, dst):
        for cb in range(3):
            q = None
            for t in range(5):
                n = 5 * cb + t
                r = mm(ylhs[t], slot[WQ0 + n // 2, pl.ds(64 * (n % 2), 64), :])
                q = r if q is None else q + r
                yield CM
            q = _rnd(q * (DH ** -0.5 * LOG2E))
            for half in range(2):
                dst[2 * cb + half] = jnp.where(same_c, expand(q, half), 0.0)

    def scores(q, h, kv, s_0, sref):
        m = None
        for j in range(NJ):
            s = None
            for t in range(3):
                r = mm(q[3 * h + t], kv[pl.ds(s_0 + 8 * t, 8), 8 * j:8 * j + 8, :])
                s = r if s is None else s + r
                yield CM
            sref[j] = s
            m = s if m is None else jnp.maximum(m, s)
        sref[NJ] = jnp.maximum(m, pltpu.roll(m, 4, 0))

    def softmax(h, sref, pref):
        m = jnp.max(sref[NJ], axis=1, keepdims=True)
        l = None
        for j in range(NJ):
            e = jnp.exp2(sref[j] - m)
            pref[j] = e
            l = e if l is None else l + e
        l = l + pltpu.roll(l, 4, 0)
        linv[h] = jnp.broadcast_to(1.0 / jnp.sum(l, axis=1, keepdims=True), (8, 128))
        yield 0

    def pv_vpu(kv, strips, pref, z0=0):
        consts = (jnp.full((8, 128), 16, I32), jnp.full((8, 128), -65536, I32))
        shift, mask = consts
        for s in strips:
            for j in range(NJ):
                w = kv[V0 + s, 8 * j:8 * j + 8, :]
                if (s, j) in WIDE:
                    a, b = vregs_of(kv, [16 * LO0 + WIDE.index((s, j))]), w
                else:
                    tied = tie(consts, LAG_V, PER_V)
                    if tied is not consts:
                        shift, mask = tied
                    a, b = w << shift, w & mask
                a = pltpu.bitcast(a, F32) * pref[j]
                b = pltpu.bitcast(b, F32) * pref[j]
                lo = a if j == 0 else lo + a
                hi = b if j == 0 else hi + b
                publish([lo, hi])
                yield 1.1 if (s, j) in WIDE else 1.6
            zbuf[0, z0 + s] = lo
            zbuf[1, z0 + s] = hi

    def lanes_to_cols(strips):
        cols = {}
        place = (lane >> 1) - (sub & 3)
        for s in strips:
            v = jnp.where((lane & 1) == 0, jnp.sum(zbuf[0, s], axis=1, keepdims=True),
                          jnp.sum(zbuf[1, s], axis=1, keepdims=True))
            cols[s // 16] = jnp.where(place == 4 * (s % 16), v, cols.get(s // 16, 0.0))
        return cols

    def finish(h, outs):
        la, lb = linv[h], linv[h + 1]
        for u, inv in enumerate((la, jnp.where(lane < 64, la, lb), lb)):
            olhs[u] = down_lhs(_rnd(outs[u] * inv))

    def finish_vpu(h):
        cols = lanes_to_cols(range(2 * HS))
        finish(h, [all_rows_sum(cols[u]) for u in range(3)])
        yield 0

    def pv_mxu(s_0, pref, res):
        for t in range(1, 3):
            acc = None
            for j in range(NJ):
                r = mm(_rnd(pref[j]), bigw[pl.ds(s_0 + 8 * t, 8), 8 * j:8 * j + 8, :], NT)
                acc = r if acc is None else acc + r
                yield 1.25 * CM
            a = jnp.where(same_c, acc, 0.0)
            a = a + pltpu.roll(a, 4, 0)
            idx = ((lane & 56) << 1) + (lane & 7)
            res.append(gather(a, idx) + gather(a, idx + 8))

    def residual(bias=None):
        ys = collect([oacc[t] for t in range(5)])
        xs = [xres[n] + ys[n] for n in range(5)]
        if bias is not None:
            xs = [xs[n] + bcast_row(bias, n) for n in range(5)]
        for n in range(5):
            xres[n] = xs[n]
            oacc[n] = jnp.zeros((8, 128), F32)
        return xs

    small = [pltpu.make_async_copy(s, d, sems.at[2])
             for s, d in ((x_hbm, xb), (b1_hbm, b1b), (b2_hbm, b2b))]
    for c in small:
        c.start()
    for half in range(2):
        issue_weight(wq_hbm, 60 * half, big, SLOT * (NP - 2 + half), 60, sems.at[3 + half])
    zeros[...] = jnp.zeros((8, 128), I32)
    for c in small:
        c.wait()
    x0 = xb[...].astype(F32)
    for n in range(5):
        xres[n] = jnp.broadcast_to(x0[:, 128 * n:128 * n + 128], (8, 128))
        oacc[n] = jnp.zeros((8, 128), F32)
    for half in range(2):
        issue_k(half, sems.at[1 - half])
        wait(big.at[pl.ds(SLOT * (NP - 2 + half), 60)], sems.at[3 + half])
        unpair_wq(half)
    issue_v_wo(0, sems.at[0])
    wait_k(0, sems.at[1])

    def slot_at(i):
        return bigw.at[pl.ds(SLOT * i, SLOT)]

    def layer(li, carry):
        first = li == 0
        ds, inv = layernorm([xres[n] for n in range(5)])
        for t in range(5):
            ylhs[t] = _rnd(ds[t] * inv)
        weave(chain(q_proj(slot_at(NP - 2), q0), q_proj(slot_at(NP - 1), q1),
                    scores(q0, 0, bigw, K0, s0), softmax(0, s0, p0),
                    scores(q0, 1, bigw, K0 + HS, s1)))
        linv[1] = jnp.zeros((8, 128), F32)
        zbuf[:, 0:2 * HS] = jnp.zeros((2, 2 * HS, 8, 128), F32)

        def step(i, c):
            @pl.when(first)
            def _():
                now, nxt = sems.at[i & 1], sems.at[1 - (i & 1)]

                @pl.when(i < NP - 2)
                def _():
                    issue_k(i + 2, nxt)
                issue_v_wo(i + 1, nxt)

                @pl.when(i == NP - 2)
                def _():
                    issue_weight(w1_hbm, 0, w1b, 0, 30, sems.at[3])
                wait_k(i + 1, now)
                wait_v_wo(i, now)
                widen_v(i)

            h = 2 * i
            kv = bigw.at[pl.ds(SLOT * i, SLOT + 2 * HS)]
            prev = jnp.maximum(h - 2, 0)
            weave(chain(scores(q1, 0, kv, SLOT, s0), scores(q1, 1, kv, SLOT + HS, s1),
                        q_proj(kv, q1), o_proj(kv)),
                  chain(finish_vpu(prev), softmax(h + 1, s1, p1), pv_vpu(kv, range(HS), p0),
                        softmax(h + 2, s0, p0), pv_vpu(kv, range(HS, 2 * HS), p1)))
            return c

        lax.fori_loop(0, NP - 1, step, 0)

        @pl.when(first)
        def _():
            issue_weight(w2_hbm, 0, w2b, 0, 30, sems.at[4])
            wait_v_wo(NP - 1, sems.at[1])
            widen_v(NP - 1, 32)

        last = []
        kv = slot_at(NP - 1)
        weave(chain(softmax(H - 1, s1, p1), finish_vpu(H - 4),
                    pv_mxu(SLOT * (NP - 1) + V0 + HS, p1, last), o_proj(kv)),
              chain(pv_vpu(kv, range(HS), p0, 2 * HS), pv_vpu(kv, range(HS, 32), p1, 2 * HS)),
              tied=False)
        cols = lanes_to_cols(range(2 * HS, 2 * HS + 32))
        finish(H - 2, [all_rows_sum(cols[3]), all_rows_sum(cols[4]),
                       jnp.where(lane < 64, last[0], last[1])])
        weave(o_proj(slot_at(0)))

        @pl.when(first)
        def _():
            weave(ffn(lambda: wait(w1b, sems.at[3]), lambda: wait(w2b, sems.at[4])))
        return carry

    def ffn(wait_w1, wait_w2):
        ds, inv = layernorm(residual())
        for t in range(10):
            ylhs[t] = jnp.where(same_c, _rnd(expand(ds[t // 2], t % 2) * inv), 0.0)
        wait_w1()
        b1 = b1b[...].astype(F32)
        for j in range(6):
            hid = jnp.where(sub < 4, bcast_row(b1, 2 * j), bcast_row(b1, 2 * j + 1))
            for t in range(10):
                hid += mm(ylhs[t], vregs_of(w1w, [6 * i + j for i in range(8 * t, 8 * t + 8)]))
            for c, v in enumerate(halves(_rnd(jax.nn.gelu(hid, approximate=True)))):
                hlhs[2 * j + c] = down_lhs(v)
        wait_w2()
        yield from down_proj(hlhs, 12, w2w, 0, 16)
        residual(b2b[...].astype(F32))

    lax.fori_loop(0, 2, layer, 0)
    weave(ffn(lambda: None, lambda: None))
    out_ref[...] = jnp.concatenate([xres[n, 0:1, :] for n in range(5)], axis=1).astype(out_ref.dtype)


@jax.jit
def pallas_interleave_layers__sliding_block_cached__dense_activation_gelu__decode_kernel(
    A_x: jax.Array,
    A_k_cache: jax.Array,
    A_v_cache: jax.Array,
    A_wq: jax.Array,
    A_wo: jax.Array,
    B_x: jax.Array,
    B_w1: jax.Array,
    B_b1: jax.Array,
    B_w2: jax.Array,
    B_b2: jax.Array,
):
    del B_x
    cache = lambda a: _tile_order(jnp.transpose(a, (0, 1, 3, 2)).reshape(H * DH, SK), SK // 16)
    args = (
        A_x.reshape(1, D), cache(A_k_cache), cache(A_v_cache),
        _tile_order(A_wq, 256), _tile_order(A_wo, 240),
        _tile_order(B_w1, 256), B_b1.reshape(F // 128, 128),
        _tile_order(B_w2, 256), B_b2.reshape(D // 128, 128),
    )
    vm = pltpu.VMEM
    vregs = lambda *n: vm((*n, 8, 128), F32)
    out = pl.pallas_call(
        _kernel,
        out_shape=jax.ShapeDtypeStruct((1, D), A_x.dtype),
        in_specs=[pl.BlockSpec(memory_space=pl.ANY)] * len(args),
        scratch_shapes=[
            vm((NP * SLOT, WROWS, 128), BF16),
            vm((30, WROWS, 128), BF16), vm((30, WROWS, 128), BF16),
            vm((1, D), BF16), vm((F // 128, 128), BF16), vm((D // 128, 128), BF16),
            vregs(5), vregs(10), vregs(12), vregs(6), vregs(6), vregs(NJ + 1), vregs(NJ + 1),
            vregs(NJ), vregs(NJ), vregs(H), vregs(2, 2 * HS + 32), vregs(3), vregs(5),
            vm((8, 128), I32),
            pltpu.SemaphoreType.DMA((5,)),
        ],
        compiler_params=pltpu.CompilerParams(
            vmem_limit_bytes=127 * 2 ** 20, disable_bounds_checks=True),
        name="interleave_decode",
    )(*args)
    return out.reshape(1, 1, D)
```

```python
import jax
import jax.numpy as jnp
from jax import lax
import jax.experimental.pallas as pl
import jax.experimental.pallas.tpu as pltpu

D, F, H, DH, SK, W = 640, 1536, 32, 192, 32768, 4096
NS = H * DH // 8
HS = DH // 8
NP = H // 2
NJ = W // 256
WIN0 = (SK - W) // 16
WROWS = W // 16
WIDE = [(s, j) for s in range(32) for j in (3, 7, 11, 15)]
K0, V0, WO0, WQ0, LO0 = 0, 2 * HS, 4 * HS, 4 * HS + 8, 4 * HS + 16
SLOT = LO0 + len(WIDE) // 16
SPLIT = 64
LAG_M, PER_M, LAG_V, PER_V = 20, 16, 150, 24
KN, KSPLIT, VN = 1, 128, 2
CM = 8.0
EPS = 1e-5
LOG2E = 1.4426950408889634
F32, BF16, I32 = jnp.float32, jnp.bfloat16, jnp.int32
NN = (((1,), (0,)), ((), ()))
NT = (((1,), (1,)), ((), ()))


def _tile_order(a, rows):
    r, c = a.shape
    a = a.reshape(r // 8, 8, c // 128, 128).transpose(0, 2, 1, 3)
    return a.reshape(-1, rows, 128)


def _rnd(x):
    return x.astype(BF16).astype(F32)


def _kernel(x_hbm, k_hbm, v_hbm, wq_hbm, wo_hbm, w1_hbm, b1_hbm, w2_hbm, b2_hbm,
            out_ref,
            big, w1b, w2b, xb, b1b, b2b,
            xres, ylhs, hlhs, q0, q1, s0, s1, p0, p1, linv, zbuf, olhs, oacc, zeros,
            sems):
    bigw = big.bitcast(I32)
    w1w, w2w = w1b.bitcast(I32), w2b.bitcast(I32)

    sub = lax.broadcasted_iota(I32, (8, 128), 0)
    lane = lax.broadcasted_iota(I32, (8, 128), 1)

    def copy(src, row0, dst, sem, split=SPLIT):
        rows = dst.shape[-2]
        for r0, n, prio in ((0, rows - split, 1), (rows - split, split, 0)):
            pltpu.make_async_copy(src.at[:, pl.ds(row0 + r0, n), :], dst.at[:, pl.ds(r0, n), :],
                                  sem).start(priority=prio)

    def issue_weight(src, src0, dst, dst0, count, sem):
        def body(t, c):
            s = jnp.where(t < count - 1, (8 * t) % (count - 1), t)
            copy(src.at[pl.ds(src0 + s, 1)], 0, dst.at[pl.ds(dst0 + s, 1)], sem)
            return c
        lax.fori_loop(0, count, body, 0)

    def issue_k(i, sem):
        def body(t, c):
            for n in range(0, 2, KN):
                copy(k_hbm.at[pl.ds(2 * HS * i + 2 * t + n, KN)], WIN0,
                     big.at[pl.ds(SLOT * i + K0 + 2 * t + n, KN)], sem, KSPLIT)
            return c
        lax.fori_loop(0, HS, body, 0)

    def issue_v_wo(i, sem):
        def body(t, c):
            copy(wo_hbm.at[pl.ds(8 * ((i + NP - 1) % NP) + t, 1)], 0,
                 big.at[pl.ds(SLOT * i + WO0 + t, 1), pl.ds(0, 240), :], sem)
            for n in range(0, 6, VN):
                copy(v_hbm.at[pl.ds(2 * HS * i + 6 * t + n, VN)], WIN0,
                     big.at[pl.ds(SLOT * i + V0 + 6 * t + n, VN)], sem)
            return c
        lax.fori_loop(0, 8, body, 0)

    def wait(ref, sem):
        pltpu.make_async_copy(ref, ref, sem).wait()

    def wait_k(i, sem):
        wait(big.at[pl.ds(SLOT * i + K0, 2 * HS)], sem)

    def wait_v_wo(i, sem):
        wait(big.at[pl.ds(SLOT * i + V0, 2 * HS)], sem)
        wait(big.at[pl.ds(SLOT * i + WO0, 8), pl.ds(0, 240), :], sem)

    def widen_v(i, strips=2 * HS):
        slot = bigw.at[pl.ds(SLOT * i, SLOT)]
        for n, (s, j) in enumerate(WIDE):
            if s < strips:
                w = slot[V0 + s, 8 * j:8 * j + 8, :]
                slot[LO0 + n // 16, pl.ds(8 * (n % 16), 8), :] = w << 16
                slot[V0 + s, 8 * j:8 * j + 8, :] = w & -65536

    def unpair_wq(half):
        def body(u, c):
            src = bigw.at[pl.ds(SLOT * (NP - 2 + half) + 3 * u, 3)]
            for j in range(24):
                a = src[j // 16, pl.ds(8 * (j % 16), 8), :]
                b = src[(24 + j) // 16, pl.ds(8 * ((24 + j) % 16), 8), :]
                both = (jnp.where(sub < 4, a, pltpu.roll(b, 4, 0)),
                        jnp.where(sub < 4, pltpu.roll(a, 4, 0), b))
                for cb, w in zip((2 * j, 2 * j + 1), both):
                    n = 40 * (cb % 3) + 20 * half + u
                    bigw[SLOT * ((cb // 3 + NP - 2) % NP) + WQ0 + (n >> 4),
                         pl.ds(pl.multiple_of(8 * (n & 15), 8), 8), :] = w
            return c
        lax.fori_loop(0, 20, body, 0)

    def bcast_row(v, r):
        return jnp.broadcast_to(v[r:r + 1, :], (8, 128))

    def halves(v):
        rolled = pltpu.roll(v, 4, 0)
        return jnp.where(sub < 4, v, rolled), jnp.where(sub < 4, rolled, v)

    def all_rows_sum(v):
        return jnp.broadcast_to(jnp.sum(v, axis=0, keepdims=True), (8, 128))

    def gather(v, idx):
        return jnp.take_along_axis(v, idx, axis=1, mode="promise_in_bounds")

    same_c = ((lane >> 3) & 1) == (sub >> 2)

    def expand(v, half):
        return gather(v, 64 * half + ((lane >> 4) << 3) + (lane & 7))

    def down_lhs(v):
        return jnp.where(same_c, gather(v, (lane & ~8) + ((sub & 2) << 2)), 0.0)

    def layernorm(xs):
        tot = xs[0] + xs[1] + xs[2] + xs[3] + xs[4]
        mean = jnp.sum(tot, axis=1, keepdims=True) * (1.0 / D)
        ds = [x - mean for x in xs]
        sq = ds[0] * ds[0] + ds[1] * ds[1] + ds[2] * ds[2] + ds[3] * ds[3] + ds[4] * ds[4]
        var = jnp.sum(sq, axis=1, keepdims=True) * (1.0 / D)
        inv = 1.0 / jnp.sqrt(var + EPS)
        return ds, inv

    def collect(outs):
        res = []
        for n in range(5):
            a, b = n, n + 5
            res.append(bcast_row(outs[a // 2], 4 * (a % 2)) + bcast_row(outs[b // 2], 4 * (b % 2) + 2))
        return res

    state = dict(me=0, clock=[0.0], toks=[[]], last=[0.0], never=None)

    def publish(v):
        state["toks"][state["me"]].append((state["clock"][state["me"]], v))

    def tie(x, lag, period):
        me = state["me"]
        now = state["clock"][me]
        if len(state["toks"]) < 2 or now - state["last"][me] < period:
            return x
        old = [v for c, v in state["toks"][1 - me] if c <= now - lag]
        if not old:
            return x
        state["last"][me] = now
        tok = sum(old[-1][1:], old[-1][0])
        return jax.tree.map(lambda a: jnp.where(state["never"], pltpu.bitcast(tok, a.dtype), a), x)

    def weave(*streams, tied=True):
        clock = [0.0] * len(streams)
        state.update(clock=clock, toks=[[] for _ in streams], last=[-1e9 if tied else 1e9] * len(streams))
        if len(streams) > 1:
            state["never"] = zeros[...] != 0
        live = list(range(len(streams)))
        while live:
            i = min(live, key=lambda n: clock[n])
            state["me"] = i
            cost = next(streams[i], None)
            if cost is None:
                live.remove(i)
            else:
                clock[i] += cost

    def chain(*gens):
        for gen in gens:
            yield from gen

    def mm(a, words, dims=NN):
        rhs = pltpu.bitcast(words.reshape(64, 128), BF16)
        r = lax.dot_general(tie(a, LAG_M, PER_M), rhs, dims, preferred_element_type=F32)
        publish([r])
        return r

    def vregs_of(ref, ns, per=16):
        return jnp.concatenate([ref[n // per, pl.ds(8 * (n % per), 8), :] for n in ns], axis=0)

    def down_proj(lhs, count, ref, n0, per):
        acc = [oacc[t] for t in range(5)]
        for n in range(count):
            for t in range(5):
                acc[t] += mm(lhs[n], vregs_of(
                    ref, [n0 + 5 * u + t for u in range(8 * n, 8 * n + 8)], per))
                yield CM
        for t in range(5):
            oacc[t] = acc[t]

    def o_proj(slot):
        return down_proj(olhs, 3, slot, 15 * WO0, 15)

    def q_proj(slot, dst):
        for cb in range(3):
            q = None
            for t in range(5):
                n = 5 * cb + t
                r = mm(ylhs[t], slot[WQ0 + n // 2, pl.ds(64 * (n % 2), 64), :])
                q = r if q is None else q + r
                yield CM
            q = _rnd(q * (DH ** -0.5 * LOG2E))
            for half in range(2):
                dst[2 * cb + half] = jnp.where(same_c, expand(q, half), 0.0)

    def scores(q, h, kv, s_0, sref):
        m = None
        for j in range(NJ):
            s = None
            for t in range(3):
                r = mm(q[3 * h + t], kv[pl.ds(s_0 + 8 * t, 8), 8 * j:8 * j + 8, :])
                s = r if s is None else s + r
                yield CM
            sref[j] = s
            m = s if m is None else jnp.maximum(m, s)
        sref[NJ] = jnp.maximum(m, pltpu.roll(m, 4, 0))

    def softmax(h, sref, pref):
        m = jnp.max(sref[NJ], axis=1, keepdims=True)
        l = None
        for j in range(NJ):
            e = jnp.exp2(sref[j] - m)
            pref[j] = e
            l = e if l is None else l + e
        l = l + pltpu.roll(l, 4, 0)
        linv[h] = jnp.broadcast_to(1.0 / jnp.sum(l, axis=1, keepdims=True), (8, 128))
        yield 0

    def pv_vpu(kv, strips, pref, z0=0):
        consts = (jnp.full((8, 128), 16, I32), jnp.full((8, 128), -65536, I32))
        shift, mask = consts
        for s in strips:
            for j in range(NJ):
                w = kv[V0 + s, 8 * j:8 * j + 8, :]
                if (s, j) in WIDE:
                    a, b = vregs_of(kv, [16 * LO0 + WIDE.index((s, j))]), w
                else:
                    tied = tie(consts, LAG_V, PER_V)
                    if tied is not consts:
                        shift, mask = tied
                    a, b = w << shift, w & mask
                a = pltpu.bitcast(a, F32) * pref[j]
                b = pltpu.bitcast(b, F32) * pref[j]
                lo = a if j == 0 else lo + a
                hi = b if j == 0 else hi + b
                publish([lo, hi])
                yield 1.1 if (s, j) in WIDE else 1.6
            zbuf[0, z0 + s] = lo
            zbuf[1, z0 + s] = hi

    def lanes_to_cols(strips):
        cols = {}
        place = (lane >> 1) - (sub & 3)
        for s in strips:
            v = jnp.where((lane & 1) == 0, jnp.sum(zbuf[0, s], axis=1, keepdims=True),
                          jnp.sum(zbuf[1, s], axis=1, keepdims=True))
            cols[s // 16] = jnp.where(place == 4 * (s % 16), v, cols.get(s // 16, 0.0))
        return cols

    def finish(h, outs):
        la, lb = linv[h], linv[h + 1]
        for u, inv in enumerate((la, jnp.where(lane < 64, la, lb), lb)):
            olhs[u] = down_lhs(_rnd(outs[u] * inv))

    def finish_vpu(h):
        cols = lanes_to_cols(range(2 * HS))
        finish(h, [all_rows_sum(cols[u]) for u in range(3)])
        yield 0

    def pv_mxu(s_0, pref, res):
        for t in range(1, 3):
            acc = None
            for j in range(NJ):
                r = mm(_rnd(pref[j]), bigw[pl.ds(s_0 + 8 * t, 8), 8 * j:8 * j + 8, :], NT)
                acc = r if acc is None else acc + r
                yield 1.25 * CM
            a = jnp.where(same_c, acc, 0.0)
            a = a + pltpu.roll(a, 4, 0)
            idx = ((lane & 56) << 1) + (lane & 7)
            res.append(gather(a, idx) + gather(a, idx + 8))

    def residual(bias=None):
        ys = collect([oacc[t] for t in range(5)])
        xs = [xres[n] + ys[n] for n in range(5)]
        if bias is not None:
            xs = [xs[n] + bcast_row(bias, n) for n in range(5)]
        for n in range(5):
            xres[n] = xs[n]
            oacc[n] = jnp.zeros((8, 128), F32)
        return xs

    small = [pltpu.make_async_copy(s, d, sems.at[2])
             for s, d in ((x_hbm, xb), (b1_hbm, b1b), (b2_hbm, b2b))]
    for c in small:
        c.start()
    for half in range(2):
        issue_weight(wq_hbm, 60 * half, big, SLOT * (NP - 2 + half), 60, sems.at[3 + half])
    zeros[...] = jnp.zeros((8, 128), I32)
    for c in small:
        c.wait()
    x0 = xb[...].astype(F32)
    for n in range(5):
        xres[n] = jnp.broadcast_to(x0[:, 128 * n:128 * n + 128], (8, 128))
        oacc[n] = jnp.zeros((8, 128), F32)
    for half in range(2):
        issue_k(half, sems.at[1 - half])
        wait(big.at[pl.ds(SLOT * (NP - 2 + half), 60)], sems.at[3 + half])
        unpair_wq(half)
    issue_v_wo(0, sems.at[0])
    wait_k(0, sems.at[1])

    def slot_at(i):
        return bigw.at[pl.ds(SLOT * i, SLOT)]

    def layer(li, carry):
        first = li == 0
        ds, inv = layernorm([xres[n] for n in range(5)])
        for t in range(5):
            ylhs[t] = _rnd(ds[t] * inv)
        weave(chain(q_proj(slot_at(NP - 2), q0), q_proj(slot_at(NP - 1), q1),
                    scores(q0, 0, bigw, K0, s0), softmax(0, s0, p0),
                    scores(q0, 1, bigw, K0 + HS, s1)))
        linv[1] = jnp.zeros((8, 128), F32)
        zbuf[:, 0:2 * HS] = jnp.zeros((2, 2 * HS, 8, 128), F32)

        def step(i, c):
            @pl.when(first)
            def _():
                now, nxt = sems.at[i & 1], sems.at[1 - (i & 1)]

                @pl.when(i < NP - 2)
                def _():
                    issue_k(i + 2, nxt)
                issue_v_wo(i + 1, nxt)

                @pl.when(i == NP - 2)
                def _():
                    issue_weight(w1_hbm, 0, w1b, 0, 30, sems.at[3])
                wait_k(i + 1, now)
                wait_v_wo(i, now)
                widen_v(i)

            h = 2 * i
            kv = bigw.at[pl.ds(SLOT * i, SLOT + 2 * HS)]
            prev = jnp.maximum(h - 2, 0)
            weave(chain(scores(q1, 0, kv, SLOT, s0), scores(q1, 1, kv, SLOT + HS, s1),
                        q_proj(kv, q1), o_proj(kv)),
                  chain(finish_vpu(prev), softmax(h + 1, s1, p1), pv_vpu(kv, range(HS), p0),
                        softmax(h + 2, s0, p0), pv_vpu(kv, range(HS, 2 * HS), p1)))
            return c

        lax.fori_loop(0, NP - 1, step, 0)

        @pl.when(first)
        def _():
            issue_weight(w2_hbm, 0, w2b, 0, 30, sems.at[4])
            wait_v_wo(NP - 1, sems.at[1])
            widen_v(NP - 1, 32)

        last = []
        kv = slot_at(NP - 1)
        weave(chain(softmax(H - 1, s1, p1), finish_vpu(H - 4),
                    pv_mxu(SLOT * (NP - 1) + V0 + HS, p1, last), o_proj(kv)),
              chain(pv_vpu(kv, range(HS), p0, 2 * HS), pv_vpu(kv, range(HS, 32), p1, 2 * HS)),
              tied=False)
        cols = lanes_to_cols(range(2 * HS, 2 * HS + 32))
        finish(H - 2, [all_rows_sum(cols[3]), all_rows_sum(cols[4]),
                       jnp.where(lane < 64, last[0], last[1])])
        weave(o_proj(slot_at(0)))

        @pl.when(first)
        def _():
            weave(ffn(lambda: wait(w1b, sems.at[3]), lambda: wait(w2b, sems.at[4])))
        return carry

    def ffn(wait_w1, wait_w2):
        ds, inv = layernorm(residual())
        for t in range(10):
            ylhs[t] = jnp.where(same_c, _rnd(expand(ds[t // 2], t % 2) * inv), 0.0)
        wait_w1()
        b1 = b1b[...].astype(F32)
        for j in range(6):
            hid = jnp.where(sub < 4, bcast_row(b1, 2 * j), bcast_row(b1, 2 * j + 1))
            for t in range(10):
                hid += mm(ylhs[t], vregs_of(w1w, [6 * i + j for i in range(8 * t, 8 * t + 8)]))
            for c, v in enumerate(halves(_rnd(jax.nn.gelu(hid, approximate=True)))):
                hlhs[2 * j + c] = down_lhs(v)
        wait_w2()
        yield from down_proj(hlhs, 12, w2w, 0, 16)
        residual(b2b[...].astype(F32))

    lax.fori_loop(0, 2, layer, 0)
    weave(ffn(lambda: None, lambda: None))
    out_ref[...] = jnp.concatenate([xres[n, 0:1, :] for n in range(5)], axis=1).astype(out_ref.dtype)


@jax.jit
def pallas_interleave_layers__sliding_block_cached__dense_activation_gelu__decode_kernel(
    A_x: jax.Array,
    A_k_cache: jax.Array,
    A_v_cache: jax.Array,
    A_wq: jax.Array,
    A_wo: jax.Array,
    B_x: jax.Array,
    B_w1: jax.Array,
    B_b1: jax.Array,
    B_w2: jax.Array,
    B_b2: jax.Array,
):
    del B_x
    cache = lambda a: _tile_order(jnp.transpose(a, (0, 1, 3, 2)).reshape(H * DH, SK), SK // 16)
    args = (
        A_x.reshape(1, D), cache(A_k_cache), cache(A_v_cache),
        _tile_order(A_wq, 256), _tile_order(A_wo, 240),
        _tile_order(B_w1, 256), B_b1.reshape(F // 128, 128),
        _tile_order(B_w2, 256), B_b2.reshape(D // 128, 128),
    )
    vm = pltpu.VMEM
    vregs = lambda *n: vm((*n, 8, 128), F32)
    out = pl.pallas_call(
        _kernel,
        out_shape=jax.ShapeDtypeStruct((1, D), A_x.dtype),
        in_specs=[pl.BlockSpec(memory_space=pl.ANY)] * len(args),
        scratch_shapes=[
            vm((NP * SLOT, WROWS, 128), BF16),
            vm((30, WROWS, 128), BF16), vm((30, WROWS, 128), BF16),
            vm((1, D), BF16), vm((F // 128, 128), BF16), vm((D // 128, 128), BF16),
            vregs(5), vregs(10), vregs(12), vregs(6), vregs(6), vregs(NJ + 1), vregs(NJ + 1),
            vregs(NJ), vregs(NJ), vregs(H), vregs(2, 2 * HS + 32), vregs(3), vregs(5),
            vm((8, 128), I32),
            pltpu.SemaphoreType.DMA((5,)),
        ],
        compiler_params=pltpu.CompilerParams(
            vmem_limit_bytes=127 * 2 ** 20, disable_bounds_checks=True),
        name="interleave_decode",
    )(*args)
    return out.reshape(1, 1, D)
```

```python
import jax
import jax.numpy as jnp
from jax import lax
import jax.experimental.pallas as pl
import jax.experimental.pallas.tpu as pltpu

D, F, H, DH, SK, W = 640, 1536, 32, 192, 32768, 4096
NS = H * DH // 8
HS = DH // 8
NP = H // 2
NJ = W // 256
WIN0 = (SK - W) // 16
WROWS = W // 16
WIDE = [(s, j) for s in range(32) for j in (3, 7, 11, 15)]
K0, V0, WO0, WQ0, LO0 = 0, 2 * HS, 4 * HS, 4 * HS + 8, 4 * HS + 16
SLOT = LO0 + len(WIDE) // 16
SPLIT = 64
LAG_M, PER_M, LAG_V, PER_V = 20, 16, 150, 24
KN, KSPLIT, VN = 1, 128, 2
CM = 8.0
EPS = 1e-5
LOG2E = 1.4426950408889634
F32, BF16, I32 = jnp.float32, jnp.bfloat16, jnp.int32
NN = (((1,), (0,)), ((), ()))
NT = (((1,), (1,)), ((), ()))


def _tile_order(a, rows):
    r, c = a.shape
    a = a.reshape(r // 8, 8, c // 128, 128).transpose(0, 2, 1, 3)
    return a.reshape(-1, rows, 128)


def _rnd(x):
    return x.astype(BF16).astype(F32)


def _kernel(x_hbm, k_hbm, v_hbm, wq_hbm, wo_hbm, w1_hbm, b1_hbm, w2_hbm, b2_hbm,
            out_ref,
            big, w1b, w2b, xb, b1b, b2b,
            xres, ylhs, hlhs, q0, q1, s0, s1, p0, p1, linv, zbuf, olhs, oacc, zeros,
            sems):
    bigw = big.bitcast(I32)
    w1w, w2w = w1b.bitcast(I32), w2b.bitcast(I32)

    sub = lax.broadcasted_iota(I32, (8, 128), 0)
    lane = lax.broadcasted_iota(I32, (8, 128), 1)

    def copy(src, row0, dst, sem, split=SPLIT):
        rows = dst.shape[-2]
        for r0, n, prio in ((0, rows - split, 1), (rows - split, split, 0)):
            pltpu.make_async_copy(src.at[:, pl.ds(row0 + r0, n), :], dst.at[:, pl.ds(r0, n), :],
                                  sem).start(priority=prio)

    def issue_weight(src, src0, dst, dst0, count, sem):
        def body(t, c):
            s = jnp.where(t < count - 1, (8 * t) % (count - 1), t)
            copy(src.at[pl.ds(src0 + s, 1)], 0, dst.at[pl.ds(dst0 + s, 1)], sem)
            return c
        lax.fori_loop(0, count, body, 0)

    def issue_k(i, sem):
        def body(t, c):
            for n in range(0, 2, KN):
                copy(k_hbm.at[pl.ds(2 * HS * i + 2 * t + n, KN)], WIN0,
                     big.at[pl.ds(SLOT * i + K0 + 2 * t + n, KN)], sem, KSPLIT)
            return c
        lax.fori_loop(0, HS, body, 0)

    def issue_v_wo(i, sem):
        def body(t, c):
            copy(wo_hbm.at[pl.ds(8 * ((i + NP - 1) % NP) + t, 1)], 0,
                 big.at[pl.ds(SLOT * i + WO0 + t, 1), pl.ds(0, 240), :], sem)
            for n in range(0, 6, VN):
                copy(v_hbm.at[pl.ds(2 * HS * i + 6 * t + n, VN)], WIN0,
                     big.at[pl.ds(SLOT * i + V0 + 6 * t + n, VN)], sem)
            return c
        lax.fori_loop(0, 8, body, 0)

    def wait(ref, sem):
        pltpu.make_async_copy(ref, ref, sem).wait()

    def wait_k(i, sem):
        wait(big.at[pl.ds(SLOT * i + K0, 2 * HS)], sem)

    def wait_v_wo(i, sem):
        wait(big.at[pl.ds(SLOT * i + V0, 2 * HS)], sem)
        wait(big.at[pl.ds(SLOT * i + WO0, 8), pl.ds(0, 240), :], sem)

    def widen_v(i, strips=2 * HS):
        slot = bigw.at[pl.ds(SLOT * i, SLOT)]
        for n, (s, j) in enumerate(WIDE):
            if s < strips:
                w = slot[V0 + s, 8 * j:8 * j + 8, :]
                slot[LO0 + n // 16, pl.ds(8 * (n % 16), 8), :] = w << 16
                slot[V0 + s, 8 * j:8 * j + 8, :] = w & -65536

    def unpair_wq(half):
        def body(u, c):
            src = bigw.at[pl.ds(SLOT * (NP - 2 + half) + 3 * u, 3)]
            for j in range(24):
                a = src[j // 16, pl.ds(8 * (j % 16), 8), :]
                b = src[(24 + j) // 16, pl.ds(8 * ((24 + j) % 16), 8), :]
                both = (jnp.where(sub < 4, a, pltpu.roll(b, 4, 0)),
                        jnp.where(sub < 4, pltpu.roll(a, 4, 0), b))
                for cb, w in zip((2 * j, 2 * j + 1), both):
                    n = 40 * (cb % 3) + 20 * half + u
                    bigw[SLOT * ((cb // 3 + NP - 2) % NP) + WQ0 + (n >> 4),
                         pl.ds(pl.multiple_of(8 * (n & 15), 8), 8), :] = w
            return c
        lax.fori_loop(0, 20, body, 0)

    def bcast_row(v, r):
        return jnp.broadcast_to(v[r:r + 1, :], (8, 128))

    def halves(v):
        rolled = pltpu.roll(v, 4, 0)
        return jnp.where(sub < 4, v, rolled), jnp.where(sub < 4, rolled, v)

    def all_rows_sum(v):
        return jnp.broadcast_to(jnp.sum(v, axis=0, keepdims=True), (8, 128))

    def gather(v, idx):
        return jnp.take_along_axis(v, idx, axis=1, mode="promise_in_bounds")

    same_c = ((lane >> 3) & 1) == (sub >> 2)

    def expand(v, half):
        return gather(v, 64 * half + ((lane >> 4) << 3) + (lane & 7))

    def down_lhs(v):
        return jnp.where(same_c, gather(v, (lane & ~8) + ((sub & 2) << 2)), 0.0)

    def layernorm(xs):
        tot = xs[0] + xs[1] + xs[2] + xs[3] + xs[4]
        mean = jnp.sum(tot, axis=1, keepdims=True) * (1.0 / D)
        ds = [x - mean for x in xs]
        sq = ds[0] * ds[0] + ds[1] * ds[1] + ds[2] * ds[2] + ds[3] * ds[3] + ds[4] * ds[4]
        var = jnp.sum(sq, axis=1, keepdims=True) * (1.0 / D)
        inv = 1.0 / jnp.sqrt(var + EPS)
        return ds, inv

    def collect(outs):
        res = []
        for n in range(5):
            a, b = n, n + 5
            res.append(bcast_row(outs[a // 2], 4 * (a % 2)) + bcast_row(outs[b // 2], 4 * (b % 2) + 2))
        return res

    state = dict(me=0, clock=[0.0], toks=[[]], last=[0.0], never=None)

    def publish(v):
        state["toks"][state["me"]].append((state["clock"][state["me"]], v))

    def tie(x, lag, period):
        me = state["me"]
        now = state["clock"][me]
        if len(state["toks"]) < 2 or now - state["last"][me] < period:
            return x
        old = [v for c, v in state["toks"][1 - me] if c <= now - lag]
        if not old:
            return x
        state["last"][me] = now
        tok = sum(old[-1][1:], old[-1][0])
        return jax.tree.map(lambda a: jnp.where(state["never"], pltpu.bitcast(tok, a.dtype), a), x)

    def weave(*streams, tied=True):
        clock = [0.0] * len(streams)
        state.update(clock=clock, toks=[[] for _ in streams], last=[-1e9 if tied else 1e9] * len(streams))
        if len(streams) > 1:
            state["never"] = zeros[...] != 0
        live = list(range(len(streams)))
        while live:
            i = min(live, key=lambda n: clock[n])
            state["me"] = i
            cost = next(streams[i], None)
            if cost is None:
                live.remove(i)
            else:
                clock[i] += cost

    def chain(*gens):
        for gen in gens:
            yield from gen

    def mm(a, words, dims=NN):
        rhs = pltpu.bitcast(words.reshape(64, 128), BF16)
        r = lax.dot_general(tie(a, LAG_M, PER_M), rhs, dims, preferred_element_type=F32)
        publish([r])
        return r

    def vregs_of(ref, ns, per=16):
        return jnp.concatenate([ref[n // per, pl.ds(8 * (n % per), 8), :] for n in ns], axis=0)

    def down_proj(lhs, blocks, ref, n0, per):
        acc = [oacc[t] for t in range(5)]
        for n in blocks:
            for t in range(5):
                acc[t] += mm(lhs[n], vregs_of(
                    ref, [n0 + 5 * u + t for u in range(8 * n, 8 * n + 8)], per))
                yield CM
        for t in range(5):
            oacc[t] = acc[t]

    def o_proj(slot):
        return down_proj(olhs, range(3), slot, 15 * WO0, 15)

    def q_proj(slot, dst):
        for cb in range(3):
            q = None
            for t in range(5):
                n = 5 * cb + t
                r = mm(ylhs[t], slot[WQ0 + n // 2, pl.ds(64 * (n % 2), 64), :])
                q = r if q is None else q + r
                yield CM
            q = _rnd(q * (DH ** -0.5 * LOG2E))
            for half in range(2):
                dst[2 * cb + half] = jnp.where(same_c, expand(q, half), 0.0)

    def scores(q, h, kv, s_0, sref):
        m = None
        for j in range(NJ):
            s = None
            for t in range(3):
                r = mm(q[3 * h + t], kv[pl.ds(s_0 + 8 * t, 8), 8 * j:8 * j + 8, :])
                s = r if s is None else s + r
                yield CM
            sref[j] = s
            m = s if m is None else jnp.maximum(m, s)
        sref[NJ] = jnp.maximum(m, pltpu.roll(m, 4, 0))

    def softmax(h, sref, pref):
        m = jnp.max(sref[NJ], axis=1, keepdims=True)
        l = None
        for j in range(NJ):
            e = jnp.exp2(sref[j] - m)
            pref[j] = e
            l = e if l is None else l + e
        l = l + pltpu.roll(l, 4, 0)
        linv[h] = jnp.broadcast_to(1.0 / jnp.sum(l, axis=1, keepdims=True), (8, 128))
        yield 0

    def pv_vpu(kv, strips, pref, z0=0):
        consts = (jnp.full((8, 128), 16, I32), jnp.full((8, 128), -65536, I32))
        shift, mask = consts
        for s in strips:
            for j in range(NJ):
                w = kv[V0 + s, 8 * j:8 * j + 8, :]
                if (s, j) in WIDE:
                    a, b = vregs_of(kv, [16 * LO0 + WIDE.index((s, j))]), w
                else:
                    tied = tie(consts, LAG_V, PER_V)
                    if tied is not consts:
                        shift, mask = tied
                    a, b = w << shift, w & mask
                a = pltpu.bitcast(a, F32) * pref[j]
                b = pltpu.bitcast(b, F32) * pref[j]
                lo = a if j == 0 else lo + a
                hi = b if j == 0 else hi + b
                publish([lo, hi])
                yield 1.1 if (s, j) in WIDE else 1.6
            zbuf[0, z0 + s] = lo
            zbuf[1, z0 + s] = hi

    def lanes_to_cols(strips):
        cols = {}
        place = (lane >> 1) - (sub & 3)
        for s in strips:
            v = jnp.where((lane & 1) == 0, jnp.sum(zbuf[0, s], axis=1, keepdims=True),
                          jnp.sum(zbuf[1, s], axis=1, keepdims=True))
            cols[s // 16] = jnp.where(place == 4 * (s % 16), v, cols.get(s // 16, 0.0))
        return cols

    def finish(h, outs):
        la, lb = linv[h], linv[h + 1]
        for u, inv in enumerate((la, jnp.where(lane < 64, la, lb), lb)):
            olhs[u] = down_lhs(_rnd(outs[u] * inv))

    def finish_step(h):
        cols = lanes_to_cols(range(2 * HS))
        finish(h, [all_rows_sum(cols[u]) for u in range(3)])
        yield 0

    def pv_mxu(kv, s_0, pref, res):
        acc = None
        for j in range(NJ):
            r = mm(_rnd(pref[j]), kv[pl.ds(V0 + s_0, 8), 8 * j:8 * j + 8, :], NT)
            acc = r if acc is None else acc + r
            yield 1.25 * CM
        a = jnp.where(same_c, acc, 0.0)
        a = a + pltpu.roll(a, 4, 0)
        idx = ((lane & 56) << 1) + (lane & 7)
        res.append(gather(a, idx) + gather(a, idx + 8))

    def residual(bias=None):
        ys = collect([oacc[t] for t in range(5)])
        xs = [xres[n] + ys[n] for n in range(5)]
        if bias is not None:
            xs = [xs[n] + bcast_row(bias, n) for n in range(5)]
        for n in range(5):
            xres[n] = xs[n]
            oacc[n] = jnp.zeros((8, 128), F32)
        return xs

    small = [pltpu.make_async_copy(s, d, sems.at[2])
             for s, d in ((x_hbm, xb), (b1_hbm, b1b), (b2_hbm, b2b))]
    for c in small:
        c.start()
    for half in range(2):
        issue_weight(wq_hbm, 60 * half, big, SLOT * (NP - 2 + half), 60, sems.at[3 + half])
    zeros[...] = jnp.zeros((8, 128), I32)
    for c in small:
        c.wait()
    x0 = xb[...].astype(F32)
    for n in range(5):
        xres[n] = jnp.broadcast_to(x0[:, 128 * n:128 * n + 128], (8, 128))
        oacc[n] = jnp.zeros((8, 128), F32)
    for half in range(2):
        issue_k(half, sems.at[1 - half])
        wait(big.at[pl.ds(SLOT * (NP - 2 + half), 60)], sems.at[3 + half])
        unpair_wq(half)
    issue_v_wo(0, sems.at[0])
    wait_k(0, sems.at[1])

    def slot_at(i):
        return bigw.at[pl.ds(SLOT * i, SLOT)]

    def layer(li, carry):
        first = li == 0
        ds, inv = layernorm([xres[n] for n in range(5)])
        for t in range(5):
            ylhs[t] = _rnd(ds[t] * inv)
        weave(chain(q_proj(slot_at(NP - 2), q0), q_proj(slot_at(NP - 1), q1),
                    scores(q0, 0, bigw, K0, s0), softmax(0, s0, p0),
                    scores(q0, 1, bigw, K0 + HS, s1)))
        linv[1] = jnp.zeros((8, 128), F32)
        zbuf[:, 0:2 * HS] = jnp.zeros((2, 2 * HS, 8, 128), F32)

        def step(i, c):
            @pl.when(first)
            def _():
                now, nxt = sems.at[i & 1], sems.at[1 - (i & 1)]

                @pl.when(i < NP - 2)
                def _():
                    issue_k(i + 2, nxt)
                issue_v_wo(i + 1, nxt)

                @pl.when(i == NP - 2)
                def _():
                    issue_weight(w1_hbm, 0, w1b, 0, 30, sems.at[3])
                wait_k(i + 1, now)
                wait_v_wo(i, now)
                widen_v(i)

            h = 2 * i
            kv = bigw.at[pl.ds(SLOT * i, SLOT + 2 * HS)]
            prev = jnp.maximum(h - 2, 0)
            weave(chain(finish_step(prev), softmax(h + 1, s1, p1), pv_vpu(kv, range(HS), p0),
                        softmax(h + 2, s0, p0), pv_vpu(kv, range(HS, 2 * HS), p1)),
                  chain(scores(q1, 0, kv, SLOT, s0), scores(q1, 1, kv, SLOT + HS, s1),
                        q_proj(kv, q1), o_proj(kv)))
            return c

        lax.fori_loop(0, NP - 1, step, 0)

        @pl.when(first)
        def _():
            issue_weight(w2_hbm, 0, w2b, 0, 26, sems.at[4])
            issue_weight(w2_hbm, 26, w2b, 26, 4, sems.at[2])
            wait_v_wo(NP - 1, sems.at[1])
            widen_v(NP - 1, 32)

        kv, last = slot_at(NP - 1), []
        weave(chain(softmax(H - 1, s1, p1), finish_step(H - 4), pv_mxu(kv, 32, p1, last),
                    pv_mxu(kv, 40, p1, last), o_proj(kv)),
              chain(pv_vpu(kv, range(HS), p0, 2 * HS), pv_vpu(kv, range(HS, 32), p1, 2 * HS)),
              tied=False)
        cols = lanes_to_cols(range(2 * HS, 2 * HS + 32))
        finish(H - 2, [all_rows_sum(cols[3]), all_rows_sum(cols[4]),
                       jnp.where(lane < 64, last[0], last[1])])
        weave(o_proj(slot_at(0)))

        @pl.when(first)
        def _():
            weave(ffn(wait))
        return carry

    def ffn(arrived):
        ds, inv = layernorm(residual())
        for t in range(10):
            ylhs[t] = jnp.where(same_c, _rnd(expand(ds[t // 2], t % 2) * inv), 0.0)
        arrived(w1b, sems.at[3])
        b1 = b1b[...].astype(F32)
        for j in range(6):
            hid = jnp.where(sub < 4, bcast_row(b1, 2 * j), bcast_row(b1, 2 * j + 1))
            for t in range(10):
                hid += mm(ylhs[t], vregs_of(w1w, [6 * i + j for i in range(8 * t, 8 * t + 8)]))
            for c, v in enumerate(halves(_rnd(jax.nn.gelu(hid, approximate=True)))):
                hlhs[2 * j + c] = down_lhs(v)
        arrived(w2b.at[0:26], sems.at[4])
        yield from down_proj(hlhs, range(10), w2w, 0, 16)
        arrived(w2b.at[26:30], sems.at[2])
        yield from down_proj(hlhs, range(10, 12), w2w, 0, 16)
        residual(b2b[...].astype(F32))

    lax.fori_loop(0, 2, layer, 0)
    weave(ffn(lambda ref, sem: None))
    out_ref[...] = jnp.concatenate([xres[n, 0:1, :] for n in range(5)], axis=1).astype(out_ref.dtype)


@jax.jit
def pallas_interleave_layers__sliding_block_cached__dense_activation_gelu__decode_kernel(
    A_x: jax.Array,
    A_k_cache: jax.Array,
    A_v_cache: jax.Array,
    A_wq: jax.Array,
    A_wo: jax.Array,
    B_x: jax.Array,
    B_w1: jax.Array,
    B_b1: jax.Array,
    B_w2: jax.Array,
    B_b2: jax.Array,
):
    del B_x
    cache = lambda a: _tile_order(jnp.transpose(a, (0, 1, 3, 2)).reshape(H * DH, SK), SK // 16)
    args = (
        A_x.reshape(1, D), cache(A_k_cache), cache(A_v_cache),
        _tile_order(A_wq, 256), _tile_order(A_wo, 240),
        _tile_order(B_w1, 256), B_b1.reshape(F // 128, 128),
        _tile_order(B_w2, 256), B_b2.reshape(D // 128, 128),
    )
    vm = pltpu.VMEM
    vregs = lambda *n: vm((*n, 8, 128), F32)
    out = pl.pallas_call(
        _kernel,
        out_shape=jax.ShapeDtypeStruct((1, D), A_x.dtype),
        in_specs=[pl.BlockSpec(memory_space=pl.ANY)] * len(args),
        scratch_shapes=[
            vm((NP * SLOT, WROWS, 128), BF16),
            vm((30, WROWS, 128), BF16), vm((30, WROWS, 128), BF16),
            vm((1, D), BF16), vm((F // 128, 128), BF16), vm((D // 128, 128), BF16),
            vregs(5), vregs(10), vregs(12), vregs(6), vregs(6), vregs(NJ + 1), vregs(NJ + 1),
            vregs(NJ), vregs(NJ), vregs(H), vregs(2, 2 * HS + 32), vregs(3), vregs(5),
            vm((8, 128), I32),
            pltpu.SemaphoreType.DMA((5,)),
        ],
        compiler_params=pltpu.CompilerParams(
            vmem_limit_bytes=127 * 2 ** 20, disable_bounds_checks=True),
        name="interleave_decode",
    )(*args)
    return out.reshape(1, 1, D)
```

```python
import jax
import jax.numpy as jnp
from jax import lax
import jax.experimental.pallas as pl
import jax.experimental.pallas.tpu as pltpu

D, F, H, DH, SK, W = 640, 1536, 32, 192, 32768, 4096
HS = DH // 8
NP = H // 2
NJ = W // 256
WIN0 = (SK - W) // 16
WROWS = W // 16
WIDE = [(s, j) for s in range(32) for j in (3, 7, 11, 15)]
K0, V0, WO0, WQ0, LO0 = 0, 2 * HS, 4 * HS, 4 * HS + 8, 4 * HS + 16
SLOT = LO0 + len(WIDE) // 16
SPLIT, SPLIT_K = 64, 128
CM = 8.0
LAG_M, PER_M, LAG_V, PER_V = 20, 16, 150, 24
EPS = 1e-5
LOG2E = 1.4426950408889634
F32, BF16, I32 = jnp.float32, jnp.bfloat16, jnp.int32
NN = (((1,), (0,)), ((), ()))
NT = (((1,), (1,)), ((), ()))


def _tile_order(a, rows):
    r, c = a.shape
    a = a.reshape(r // 8, 8, c // 128, 128).transpose(0, 2, 1, 3)
    return a.reshape(-1, rows, 128)


def _rnd(x):
    return x.astype(BF16).astype(F32)


def _kernel(x_hbm, k_hbm, v_hbm, wq_hbm, wo_hbm, w1_hbm, b1_hbm, w2_hbm, b2_hbm,
            out_ref,
            big, w1b, w2b, xb, b1b, b2b,
            xres, ylhs, hlhs, q0, q1, s0, s1, p0, p1, linv, zbuf, olhs, oacc, zeros,
            sems, ksem, vsem, osem):
    bigw = big.bitcast(I32)
    w1w, w2w = w1b.bitcast(I32), w2b.bitcast(I32)

    sub = lax.broadcasted_iota(I32, (8, 128), 0)
    lane = lax.broadcasted_iota(I32, (8, 128), 1)

    def copy(src, row0, dst, sem, split=SPLIT):
        rows = dst.shape[-2]
        for r0, n, prio in ((0, rows - split, 1), (rows - split, split, 0)):
            pltpu.make_async_copy(src.at[:, pl.ds(row0 + r0, n), :], dst.at[:, pl.ds(r0, n), :],
                                  sem).start(priority=prio)

    def issue_weight(src, src0, dst, dst0, count, sem):
        def body(t, c):
            s = jnp.where(t < count - 1, (8 * t) % (count - 1), t)
            copy(src.at[pl.ds(src0 + s, 1)], 0, dst.at[pl.ds(dst0 + s, 1)], sem)
            return c
        lax.fori_loop(0, count, body, 0)

    def issue_k(i):
        def body(t, c):
            for n in range(2):
                copy(k_hbm.at[pl.ds(2 * HS * i + 2 * t + n, 1)], WIN0,
                     big.at[pl.ds(SLOT * i + K0 + 2 * t + n, 1)], ksem.at[i & 1], SPLIT_K)
            return c
        lax.fori_loop(0, HS, body, 0)

    def issue_v_wo(i):
        def body(t, c):
            copy(wo_hbm.at[pl.ds(8 * ((i + NP - 1) & (NP - 1)) + t, 1)], 0,
                 big.at[pl.ds(SLOT * i + WO0 + t, 1), pl.ds(0, 240), :], osem.at[i & 1])
            for n in range(0, 6, 2):
                copy(v_hbm.at[pl.ds(2 * HS * i + 6 * t + n, 2)], WIN0,
                     big.at[pl.ds(SLOT * i + V0 + 6 * t + n, 2)], vsem.at[i & 1])
            return c
        lax.fori_loop(0, 8, body, 0)

    def wait(ref, sem):
        pltpu.make_async_copy(ref, ref, sem).wait()

    def wait_k(i):
        wait(big.at[pl.ds(SLOT * i + K0, 2 * HS)], ksem.at[i & 1])

    def wait_v_wo(i):
        wait(big.at[pl.ds(SLOT * i + V0, 2 * HS)], vsem.at[i & 1])
        wait(big.at[pl.ds(SLOT * i + WO0, 8), pl.ds(0, 240), :], osem.at[i & 1])

    def widen_v(i, strips=2 * HS):
        slot = bigw.at[pl.ds(SLOT * i, SLOT)]
        for n, (s, j) in enumerate(WIDE):
            if s < strips:
                w = slot[V0 + s, 8 * j:8 * j + 8, :]
                slot[LO0 + n // 16, pl.ds(8 * (n % 16), 8), :] = w << 16
                slot[V0 + s, 8 * j:8 * j + 8, :] = w & -65536

    def unpair_wq(half):
        def body(u, c):
            src = bigw.at[pl.ds(SLOT * (NP - 2 + half) + 3 * u, 3)]
            for j in range(24):
                a = src[j // 16, pl.ds(8 * (j % 16), 8), :]
                b = src[(24 + j) // 16, pl.ds(8 * ((24 + j) % 16), 8), :]
                both = (jnp.where(sub < 4, a, pltpu.roll(b, 4, 0)),
                        jnp.where(sub < 4, pltpu.roll(a, 4, 0), b))
                for cb, w in zip((2 * j, 2 * j + 1), both):
                    n = 40 * (cb % 3) + 20 * half + u
                    bigw[SLOT * ((cb // 3 + NP - 2) % NP) + WQ0 + (n >> 4),
                         pl.ds(pl.multiple_of(8 * (n & 15), 8), 8), :] = w
            return c
        lax.fori_loop(0, 20, body, 0)

    def bcast_row(v, r):
        return jnp.broadcast_to(v[r:r + 1, :], (8, 128))

    def halves(v):
        rolled = pltpu.roll(v, 4, 0)
        return jnp.where(sub < 4, v, rolled), jnp.where(sub < 4, rolled, v)

    def all_rows_sum(v):
        return jnp.broadcast_to(jnp.sum(v, axis=0, keepdims=True), (8, 128))

    def gather(v, idx):
        return jnp.take_along_axis(v, idx, axis=1, mode="promise_in_bounds")

    same_c = ((lane >> 3) & 1) == (sub >> 2)

    def expand(v, half):
        return gather(v, 64 * half + ((lane >> 4) << 3) + (lane & 7))

    def down_lhs(v):
        return jnp.where(same_c, gather(v, (lane & ~8) + ((sub & 2) << 2)), 0.0)

    def layernorm(xs):
        tot = xs[0] + xs[1] + xs[2] + xs[3] + xs[4]
        mean = jnp.sum(tot, axis=1, keepdims=True) * (1.0 / D)
        ds = [x - mean for x in xs]
        sq = ds[0] * ds[0] + ds[1] * ds[1] + ds[2] * ds[2] + ds[3] * ds[3] + ds[4] * ds[4]
        var = jnp.sum(sq, axis=1, keepdims=True) * (1.0 / D)
        inv = 1.0 / jnp.sqrt(var + EPS)
        return ds, inv

    def collect(outs):
        res = []
        for n in range(5):
            a, b = n, n + 5
            res.append(bcast_row(outs[a // 2], 4 * (a % 2)) + bcast_row(outs[b // 2], 4 * (b % 2) + 2))
        return res

    state = dict(me=0, clock=[0.0], toks=[[]], last=[0.0], never=None)

    def publish(v):
        state["toks"][state["me"]].append((state["clock"][state["me"]], v))

    def tie(x, lag, period):
        me = state["me"]
        now = state["clock"][me]
        if len(state["toks"]) < 2 or now - state["last"][me] < period:
            return x
        old = [v for c, v in state["toks"][1 - me] if c <= now - lag]
        if not old:
            return x
        state["last"][me] = now
        tok = sum(old[-1][1:], old[-1][0])
        return jax.tree.map(lambda a: jnp.where(state["never"], pltpu.bitcast(tok, a.dtype), a), x)

    def weave(*streams, tied=True):
        clock = [0.0] * len(streams)
        state.update(clock=clock, toks=[[] for _ in streams],
                     last=[-1e9 if tied else 1e9] * len(streams))
        if len(streams) > 1:
            state["never"] = zeros[...] != 0
        live = list(range(len(streams)))
        while live:
            i = min(live, key=lambda n: clock[n])
            state["me"] = i
            cost = next(streams[i], None)
            if cost is None:
                live.remove(i)
            else:
                clock[i] += cost

    def chain(*gens):
        for gen in gens:
            yield from gen

    def mm(a, words, dims=NN):
        rhs = pltpu.bitcast(words.reshape(64, 128), BF16)
        r = lax.dot_general(tie(a, LAG_M, PER_M), rhs, dims, preferred_element_type=F32)
        publish([r])
        return r

    def vregs_of(ref, ns, per=16):
        return jnp.concatenate([ref[n // per, pl.ds(8 * (n % per), 8), :] for n in ns], axis=0)

    def down_proj(lhs, blocks, ref, n0, per):
        acc = [oacc[t] for t in range(5)]
        for n in blocks:
            for t in range(5):
                acc[t] += mm(lhs[n], vregs_of(
                    ref, [n0 + 5 * u + t for u in range(8 * n, 8 * n + 8)], per))
                yield CM
        for t in range(5):
            oacc[t] = acc[t]

    def o_proj(slot):
        return down_proj(olhs, range(3), slot, 15 * WO0, 15)

    def q_proj(slot, dst):
        for cb in range(3):
            q = None
            for t in range(5):
                n = 5 * cb + t
                r = mm(ylhs[t], slot[WQ0 + n // 2, pl.ds(64 * (n % 2), 64), :])
                q = r if q is None else q + r
                yield CM
            q = _rnd(q * (DH ** -0.5 * LOG2E))
            for half in range(2):
                dst[2 * cb + half] = jnp.where(same_c, expand(q, half), 0.0)

    def scores(q, h, kv, s_0, sref):
        m = None
        for j in range(NJ):
            s = None
            for t in range(3):
                r = mm(q[3 * h + t], kv[pl.ds(s_0 + 8 * t, 8), 8 * j:8 * j + 8, :])
                s = r if s is None else s + r
                yield CM
            sref[j] = s
            m = s if m is None else jnp.maximum(m, s)
        sref[NJ] = jnp.maximum(m, pltpu.roll(m, 4, 0))

    def softmax(h, sref, pref):
        m = jnp.max(sref[NJ], axis=1, keepdims=True)
        l = None
        for j in range(NJ):
            e = jnp.exp2(sref[j] - m)
            pref[j] = e
            l = e if l is None else l + e
        l = l + pltpu.roll(l, 4, 0)
        linv[h] = jnp.broadcast_to(1.0 / jnp.sum(l, axis=1, keepdims=True), (8, 128))
        yield 0

    def pv_vpu(kv, strips, pref, z0=0):
        consts = (jnp.full((8, 128), 16, I32), jnp.full((8, 128), -65536, I32))
        shift, mask = consts
        for s in strips:
            for j in range(NJ):
                w = kv[V0 + s, 8 * j:8 * j + 8, :]
                if (s, j) in WIDE:
                    a, b = vregs_of(kv, [16 * LO0 + WIDE.index((s, j))]), w
                else:
                    tied = tie(consts, LAG_V, PER_V)
                    if tied is not consts:
                        shift, mask = tied
                    a, b = w << shift, w & mask
                a = pltpu.bitcast(a, F32) * pref[j]
                b = pltpu.bitcast(b, F32) * pref[j]
                lo = a if j == 0 else lo + a
                hi = b if j == 0 else hi + b
                publish([lo, hi])
                yield 1.1 if (s, j) in WIDE else 1.6
            zbuf[0, z0 + s] = lo
            zbuf[1, z0 + s] = hi

    def lanes_to_cols(strips):
        cols = {}
        place = (lane >> 1) - (sub & 3)
        for s in strips:
            v = jnp.where((lane & 1) == 0, jnp.sum(zbuf[0, s], axis=1, keepdims=True),
                          jnp.sum(zbuf[1, s], axis=1, keepdims=True))
            cols[s // 16] = jnp.where(place == 4 * (s % 16), v, cols.get(s // 16, 0.0))
        return cols

    def finish(h, outs):
        la, lb = linv[h], linv[h + 1]
        for u, inv in enumerate((la, jnp.where(lane < 64, la, lb), lb)):
            olhs[u] = down_lhs(_rnd(outs[u] * inv))

    def finish_step(h):
        cols = lanes_to_cols(range(2 * HS))
        finish(h, [all_rows_sum(cols[u]) for u in range(3)])
        yield 0

    def pv_mxu(kv, s_0, pref, res):
        acc = None
        for j in range(NJ):
            r = mm(_rnd(pref[j]), kv[pl.ds(V0 + s_0, 8), 8 * j:8 * j + 8, :], NT)
            acc = r if acc is None else acc + r
            yield 1.25 * CM
        a = jnp.where(same_c, acc, 0.0)
        a = a + pltpu.roll(a, 4, 0)
        idx = ((lane & 56) << 1) + (lane & 7)
        res.append(gather(a, idx) + gather(a, idx + 8))

    def residual(bias=None):
        ys = collect([oacc[t] for t in range(5)])
        xs = [xres[n] + ys[n] for n in range(5)]
        if bias is not None:
            xs = [xs[n] + bcast_row(bias, n) for n in range(5)]
        for n in range(5):
            xres[n] = xs[n]
            oacc[n] = jnp.zeros((8, 128), F32)
        return xs

    small = [pltpu.make_async_copy(s, d, sems.at[0])
             for s, d in ((x_hbm, xb), (b1_hbm, b1b), (b2_hbm, b2b))]
    for c in small:
        c.start()
    for half in range(2):
        issue_weight(wq_hbm, 60 * half, big, SLOT * (NP - 2 + half), 60, sems.at[1 + half])
    zeros[...] = jnp.zeros((8, 128), I32)
    for c in small:
        c.wait()
    x0 = xb[...].astype(F32)
    for n in range(5):
        xres[n] = jnp.broadcast_to(x0[:, 128 * n:128 * n + 128], (8, 128))
        oacc[n] = jnp.zeros((8, 128), F32)
    for half in range(2):
        issue_k(half)
        wait(big.at[pl.ds(SLOT * (NP - 2 + half), 60)], sems.at[1 + half])
        unpair_wq(half)
    issue_v_wo(0)
    wait_k(0)

    def slot_at(i):
        return bigw.at[pl.ds(SLOT * i, SLOT)]

    def layer(li, carry):
        first = li == 0
        ds, inv = layernorm([xres[n] for n in range(5)])
        for t in range(5):
            ylhs[t] = _rnd(ds[t] * inv)
        weave(chain(q_proj(slot_at(NP - 2), q0), q_proj(slot_at(NP - 1), q1),
                    scores(q0, 0, bigw, K0, s0), softmax(0, s0, p0),
                    scores(q0, 1, bigw, K0 + HS, s1)))
        linv[1] = jnp.zeros((8, 128), F32)
        zbuf[:, 0:2 * HS] = jnp.zeros((2, 2 * HS, 8, 128), F32)

        def step(i, c):
            @pl.when(first)
            def _():
                @pl.when(i < NP - 2)
                def _():
                    issue_k(i + 2)
                issue_v_wo(i + 1)

                @pl.when(i == NP - 2)
                def _():
                    issue_weight(w1_hbm, 0, w1b, 0, 30, sems.at[1])
                wait_k(i + 1)
                wait_v_wo(i)
                widen_v(i)

            h = 2 * i
            kv = bigw.at[pl.ds(SLOT * i, SLOT + 2 * HS)]
            prev = jnp.maximum(h - 2, 0)
            weave(chain(finish_step(prev), softmax(h + 1, s1, p1), pv_vpu(kv, range(HS), p0),
                        softmax(h + 2, s0, p0), pv_vpu(kv, range(HS, 2 * HS), p1)),
                  chain(scores(q1, 0, kv, SLOT, s0), scores(q1, 1, kv, SLOT + HS, s1),
                        q_proj(kv, q1), o_proj(kv)))
            return c

        lax.fori_loop(0, NP - 1, step, 0)

        @pl.when(first)
        def _():
            issue_weight(w2_hbm, 0, w2b, 0, 26, sems.at[2])
            issue_weight(w2_hbm, 26, w2b, 26, 4, sems.at[0])
            wait_v_wo(NP - 1)
            widen_v(NP - 1, 32)

        kv, last = slot_at(NP - 1), []
        weave(chain(softmax(H - 1, s1, p1), finish_step(H - 4), pv_mxu(kv, 32, p1, last),
                    pv_mxu(kv, 40, p1, last), o_proj(kv)),
              chain(pv_vpu(kv, range(HS), p0, 2 * HS), pv_vpu(kv, range(HS, 32), p1, 2 * HS)),
              tied=False)
        cols = lanes_to_cols(range(2 * HS, 2 * HS + 32))
        finish(H - 2, [all_rows_sum(cols[3]), all_rows_sum(cols[4]),
                       jnp.where(lane < 64, last[0], last[1])])
        weave(o_proj(slot_at(0)))

        @pl.when(first)
        def _():
            weave(ffn(wait))
        return carry

    def ffn(arrived):
        ds, inv = layernorm(residual())
        for t in range(10):
            ylhs[t] = jnp.where(same_c, _rnd(expand(ds[t // 2], t % 2) * inv), 0.0)
        arrived(w1b, sems.at[1])
        b1 = b1b[...].astype(F32)
        for j in range(6):
            hid = jnp.where(sub < 4, bcast_row(b1, 2 * j), bcast_row(b1, 2 * j + 1))
            for t in range(10):
                hid += mm(ylhs[t], vregs_of(w1w, [6 * i + j for i in range(8 * t, 8 * t + 8)]))
            for c, v in enumerate(halves(_rnd(jax.nn.gelu(hid, approximate=True)))):
                hlhs[2 * j + c] = down_lhs(v)
        arrived(w2b.at[0:26], sems.at[2])
        yield from down_proj(hlhs, range(10), w2w, 0, 16)
        arrived(w2b.at[26:30], sems.at[0])
        yield from down_proj(hlhs, range(10, 12), w2w, 0, 16)
        residual(b2b[...].astype(F32))

    lax.fori_loop(0, 2, layer, 0)
    weave(ffn(lambda ref, sem: None))
    out_ref[...] = jnp.concatenate([xres[n, 0:1, :] for n in range(5)], axis=1).astype(out_ref.dtype)


@jax.jit
def pallas_interleave_layers__sliding_block_cached__dense_activation_gelu__decode_kernel(
    A_x: jax.Array,
    A_k_cache: jax.Array,
    A_v_cache: jax.Array,
    A_wq: jax.Array,
    A_wo: jax.Array,
    B_x: jax.Array,
    B_w1: jax.Array,
    B_b1: jax.Array,
    B_w2: jax.Array,
    B_b2: jax.Array,
):
    del B_x
    cache = lambda a: _tile_order(jnp.transpose(a, (0, 1, 3, 2)).reshape(H * DH, SK), SK // 16)
    args = (
        A_x.reshape(1, D), cache(A_k_cache), cache(A_v_cache),
        _tile_order(A_wq, 256), _tile_order(A_wo, 240),
        _tile_order(B_w1, 256), B_b1.reshape(F // 128, 128),
        _tile_order(B_w2, 256), B_b2.reshape(D // 128, 128),
    )
    vm = pltpu.VMEM
    vregs = lambda *n: vm((*n, 8, 128), F32)
    out = pl.pallas_call(
        _kernel,
        out_shape=jax.ShapeDtypeStruct((1, D), A_x.dtype),
        in_specs=[pl.BlockSpec(memory_space=pl.ANY)] * len(args),
        scratch_shapes=[
            vm((NP * SLOT, WROWS, 128), BF16),
            vm((30, WROWS, 128), BF16), vm((30, WROWS, 128), BF16),
            vm((1, D), BF16), vm((F // 128, 128), BF16), vm((D // 128, 128), BF16),
            vregs(5), vregs(10), vregs(12), vregs(6), vregs(6), vregs(NJ + 1), vregs(NJ + 1),
            vregs(NJ), vregs(NJ), vregs(H), vregs(2, 2 * HS + 32), vregs(3), vregs(5),
            vm((8, 128), I32),
            pltpu.SemaphoreType.DMA((3,)), pltpu.SemaphoreType.DMA((2,)),
            pltpu.SemaphoreType.DMA((2,)), pltpu.SemaphoreType.DMA((2,)),
        ],
        compiler_params=pltpu.CompilerParams(vmem_limit_bytes=127 * 2 ** 20),
        name="interleave_decode",
    )(*args)
    return out.reshape(1, 1, D)
```

```python
import jax
import jax.numpy as jnp
from jax import lax
import jax.experimental.pallas as pl
import jax.experimental.pallas.tpu as pltpu

D, F, H, DH, SK, W = 640, 1536, 32, 192, 32768, 4096
HS = DH // 8
NP = H // 2
NJ = W // 256
WIN0 = (SK - W) // 16
WROWS = W // 16
WIDE = [(s, j) for s in range(32) for j in (3, 7, 11, 15)]
K0, V0, WO0, WQ0, LO0 = 0, 2 * HS, 4 * HS, 4 * HS + 8, 4 * HS + 16
SLOT = LO0 + len(WIDE) // 16
SPLIT, SPLIT_K = 64, 128
CM = 8.0
LAG_M, PER_M, LAG_V, PER_V = 20, 16, 150, 24
EPS = 1e-5
LOG2E = 1.4426950408889634
F32, BF16, I32 = jnp.float32, jnp.bfloat16, jnp.int32
NN = (((1,), (0,)), ((), ()))
NT = (((1,), (1,)), ((), ()))


def _tile_order(a, rows):
    r, c = a.shape
    a = a.reshape(r // 8, 8, c // 128, 128).transpose(0, 2, 1, 3)
    return a.reshape(-1, rows, 128)


def _rnd(x):
    return x.astype(BF16).astype(F32)


def _kernel(x_hbm, k_hbm, v_hbm, wq_hbm, wo_hbm, w1_hbm, b1_hbm, w2_hbm, b2_hbm,
            out_ref,
            big, w1b, w2b, xb, b1b, b2b,
            xres, ylhs, hlhs, q0, q1, s0, s1, p0, p1, linv, zbuf, olhs, oacc, zeros,
            sems, ksem, vsem, osem):
    bigw = big.bitcast(I32)
    w1w, w2w = w1b.bitcast(I32), w2b.bitcast(I32)

    sub = lax.broadcasted_iota(I32, (8, 128), 0)
    lane = lax.broadcasted_iota(I32, (8, 128), 1)

    def copy(src, row0, dst, sem, split=SPLIT):
        rows = dst.shape[-2]
        for r0, n, prio in ((0, rows - split, 1), (rows - split, split, 0)):
            pltpu.make_async_copy(src.at[:, pl.ds(row0 + r0, n), :], dst.at[:, pl.ds(r0, n), :],
                                  sem).start(priority=prio)

    def issue_weight(src, src0, dst, dst0, count, sem):
        def body(t, c):
            s = jnp.where(t < count - 1, (8 * t) % (count - 1), t)
            copy(src.at[pl.ds(src0 + s, 1)], 0, dst.at[pl.ds(dst0 + s, 1)], sem)
            return c
        lax.fori_loop(0, count, body, 0)

    def issue_k(i):
        def body(t, c):
            for n in range(2):
                copy(k_hbm.at[pl.ds(2 * HS * i + 2 * t + n, 1)], WIN0,
                     big.at[pl.ds(SLOT * i + K0 + 2 * t + n, 1)], ksem.at[i & 1], SPLIT_K)
            return c
        lax.fori_loop(0, HS, body, 0)

    def issue_v_wo(i):
        def body(t, c):
            copy(wo_hbm.at[pl.ds(8 * ((i + NP - 1) & (NP - 1)) + t, 1)], 0,
                 big.at[pl.ds(SLOT * i + WO0 + t, 1), pl.ds(0, 240), :], osem.at[i & 1])
            for n in range(0, 6, 2):
                copy(v_hbm.at[pl.ds(2 * HS * i + 6 * t + n, 2)], WIN0,
                     big.at[pl.ds(SLOT * i + V0 + 6 * t + n, 2)], vsem.at[i & 1])
            return c
        lax.fori_loop(0, 8, body, 0)

    def wait(ref, sem):
        pltpu.make_async_copy(ref, ref, sem).wait()

    def wait_k(i):
        wait(big.at[pl.ds(SLOT * i + K0, 2 * HS)], ksem.at[i & 1])

    def wait_v_wo(i):
        wait(big.at[pl.ds(SLOT * i + V0, 2 * HS)], vsem.at[i & 1])
        wait(big.at[pl.ds(SLOT * i + WO0, 8), pl.ds(0, 240), :], osem.at[i & 1])

    def widen_v(i, strips=2 * HS):
        slot = bigw.at[pl.ds(SLOT * i, SLOT)]
        for n, (s, j) in enumerate(WIDE):
            if s < strips:
                w = slot[V0 + s, 8 * j:8 * j + 8, :]
                slot[LO0 + n // 16, pl.ds(8 * (n % 16), 8), :] = w << 16
                slot[V0 + s, 8 * j:8 * j + 8, :] = w & -65536

    def unpair_wq(half):
        def body(u, c):
            src = bigw.at[pl.ds(SLOT * (NP - 2 + half) + 3 * u, 3)]
            for j in range(24):
                a = src[j // 16, pl.ds(8 * (j % 16), 8), :]
                b = src[(24 + j) // 16, pl.ds(8 * ((24 + j) % 16), 8), :]
                both = (jnp.where(sub < 4, a, pltpu.roll(b, 4, 0)),
                        jnp.where(sub < 4, pltpu.roll(a, 4, 0), b))
                for cb, w in zip((2 * j, 2 * j + 1), both):
                    n = 40 * (cb % 3) + 20 * half + u
                    bigw[SLOT * ((cb // 3 + NP - 2) % NP) + WQ0 + (n >> 4),
                         pl.ds(pl.multiple_of(8 * (n & 15), 8), 8), :] = w
            return c
        lax.fori_loop(0, 20, body, 0)

    def bcast_row(v, r):
        return jnp.broadcast_to(v[r:r + 1, :], (8, 128))

    def halves(v):
        rolled = pltpu.roll(v, 4, 0)
        return jnp.where(sub < 4, v, rolled), jnp.where(sub < 4, rolled, v)

    def all_rows_sum(v):
        return jnp.broadcast_to(jnp.sum(v, axis=0, keepdims=True), (8, 128))

    def gather(v, idx):
        return jnp.take_along_axis(v, idx, axis=1, mode="promise_in_bounds")

    same_c = ((lane >> 3) & 1) == (sub >> 2)

    def expand(v, half):
        return gather(v, 64 * half + ((lane >> 4) << 3) + (lane & 7))

    def down_lhs(v):
        return jnp.where(same_c, gather(v, (lane & ~8) + ((sub & 2) << 2)), 0.0)

    def layernorm(xs):
        tot = xs[0] + xs[1] + xs[2] + xs[3] + xs[4]
        mean = jnp.sum(tot, axis=1, keepdims=True) * (1.0 / D)
        ds = [x - mean for x in xs]
        sq = ds[0] * ds[0] + ds[1] * ds[1] + ds[2] * ds[2] + ds[3] * ds[3] + ds[4] * ds[4]
        var = jnp.sum(sq, axis=1, keepdims=True) * (1.0 / D)
        inv = 1.0 / jnp.sqrt(var + EPS)
        return ds, inv

    def collect(outs):
        res = []
        for n in range(5):
            a, b = n, n + 5
            res.append(bcast_row(outs[a // 2], 4 * (a % 2)) + bcast_row(outs[b // 2], 4 * (b % 2) + 2))
        return res

    state = dict(me=0, clock=[0.0], toks=[[]], last=[0.0], never=None)

    def publish(v):
        state["toks"][state["me"]].append((state["clock"][state["me"]], v))

    def tie(x, lag, period):
        me = state["me"]
        now = state["clock"][me]
        if len(state["toks"]) < 2 or now - state["last"][me] < period:
            return x
        old = [v for c, v in state["toks"][1 - me] if c <= now - lag]
        if not old:
            return x
        state["last"][me] = now
        tok = sum(old[-1][1:], old[-1][0])
        return jax.tree.map(lambda a: jnp.where(state["never"], pltpu.bitcast(tok, a.dtype), a), x)

    def weave(*streams):
        clock = [0.0] * len(streams)
        state.update(clock=clock, toks=[[] for _ in streams], last=[-1e9] * len(streams))
        if len(streams) > 1:
            state["never"] = zeros[...] != 0
        live = list(range(len(streams)))
        while live:
            i = min(live, key=lambda n: clock[n])
            state["me"] = i
            cost = next(streams[i], None)
            if cost is None:
                live.remove(i)
            else:
                clock[i] += cost

    def chain(*gens):
        for gen in gens:
            yield from gen

    def mm(a, words, dims=NN):
        rhs = pltpu.bitcast(words.reshape(64, 128), BF16)
        r = lax.dot_general(tie(a, LAG_M, PER_M), rhs, dims, preferred_element_type=F32)
        publish([r])
        return r

    def vregs_of(ref, ns, per=16):
        return jnp.concatenate([ref[n // per, pl.ds(8 * (n % per), 8), :] for n in ns], axis=0)

    def down_proj(lhs, blocks, ref, n0, per):
        acc = [oacc[t] for t in range(5)]
        for n in blocks:
            for t in range(5):
                acc[t] += mm(lhs[n], vregs_of(
                    ref, [n0 + 5 * u + t for u in range(8 * n, 8 * n + 8)], per))
                yield CM
        for t in range(5):
            oacc[t] = acc[t]

    def o_proj(slot):
        return down_proj(olhs, range(3), slot, 15 * WO0, 15)

    def q_proj(slot, dst):
        for cb in range(3):
            q = None
            for t in range(5):
                n = 5 * cb + t
                r = mm(ylhs[t], slot[WQ0 + n // 2, pl.ds(64 * (n % 2), 64), :])
                q = r if q is None else q + r
                yield CM
            q = _rnd(q * (DH ** -0.5 * LOG2E))
            for half in range(2):
                dst[2 * cb + half] = jnp.where(same_c, expand(q, half), 0.0)

    def scores(q, h, kv, s_0, sref):
        m = None
        for j in range(NJ):
            s = None
            for t in range(3):
                r = mm(q[3 * h + t], kv[pl.ds(s_0 + 8 * t, 8), 8 * j:8 * j + 8, :])
                s = r if s is None else s + r
                yield CM
            sref[j] = s
            m = s if m is None else jnp.maximum(m, s)
        sref[NJ] = jnp.maximum(m, pltpu.roll(m, 4, 0))

    def softmax(h, sref, pref):
        m = jnp.max(sref[NJ], axis=1, keepdims=True)
        l = None
        for j in range(NJ):
            e = jnp.exp2(sref[j] - m)
            pref[j] = e
            l = e if l is None else l + e
        l = l + pltpu.roll(l, 4, 0)
        linv[h] = jnp.broadcast_to(1.0 / jnp.sum(l, axis=1, keepdims=True), (8, 128))
        yield 0

    def pv_vpu(kv, strips, pref, z0=0):
        consts = (jnp.full((8, 128), 16, I32), jnp.full((8, 128), -65536, I32))
        shift, mask = consts
        for s in strips:
            for j in range(NJ):
                w = kv[V0 + s, 8 * j:8 * j + 8, :]
                if (s, j) in WIDE:
                    a, b = vregs_of(kv, [16 * LO0 + WIDE.index((s, j))]), w
                else:
                    tied = tie(consts, LAG_V, PER_V)
                    if tied is not consts:
                        shift, mask = tied
                    a, b = w << shift, w & mask
                a = pltpu.bitcast(a, F32) * pref[j]
                b = pltpu.bitcast(b, F32) * pref[j]
                lo = a if j == 0 else lo + a
                hi = b if j == 0 else hi + b
                publish([lo, hi])
                yield 1.1 if (s, j) in WIDE else 1.6
            zbuf[0, z0 + s] = lo
            zbuf[1, z0 + s] = hi

    def lanes_to_cols(strips):
        cols = {}
        place = (lane >> 1) - (sub & 3)
        for s in strips:
            v = jnp.where((lane & 1) == 0, jnp.sum(zbuf[0, s], axis=1, keepdims=True),
                          jnp.sum(zbuf[1, s], axis=1, keepdims=True))
            cols[s // 16] = jnp.where(place == 4 * (s % 16), v, cols.get(s // 16, 0.0))
        return cols

    def finish(h, outs):
        la, lb = linv[h], linv[h + 1]
        for u, inv in enumerate((la, jnp.where(lane < 64, la, lb), lb)):
            olhs[u] = down_lhs(_rnd(outs[u] * inv))

    def finish_step(h):
        cols = lanes_to_cols(range(2 * HS))
        finish(h, [all_rows_sum(cols[u]) for u in range(3)])
        yield 0

    def pv_mxu(kv, s_0, pref, res):
        acc = None
        for j in range(NJ):
            r = mm(_rnd(pref[j]), kv[pl.ds(V0 + s_0, 8), 8 * j:8 * j + 8, :], NT)
            acc = r if acc is None else acc + r
            yield 1.25 * CM
        a = jnp.where(same_c, acc, 0.0)
        a = a + pltpu.roll(a, 4, 0)
        idx = ((lane & 56) << 1) + (lane & 7)
        res.append(gather(a, idx) + gather(a, idx + 8))

    def residual(bias=None):
        ys = collect([oacc[t] for t in range(5)])
        xs = [xres[n] + ys[n] for n in range(5)]
        if bias is not None:
            xs = [xs[n] + bcast_row(bias, n) for n in range(5)]
        for n in range(5):
            xres[n] = xs[n]
            oacc[n] = jnp.zeros((8, 128), F32)
        return xs

    small = [pltpu.make_async_copy(s, d, sems.at[0])
             for s, d in ((x_hbm, xb), (b1_hbm, b1b), (b2_hbm, b2b))]
    for c in small:
        c.start()
    for half in range(2):
        issue_weight(wq_hbm, 60 * half, big, SLOT * (NP - 2 + half), 60, sems.at[1 + half])
    zeros[...] = jnp.zeros((8, 128), I32)
    for c in small:
        c.wait()
    x0 = xb[...].astype(F32)
    for n in range(5):
        xres[n] = jnp.broadcast_to(x0[:, 128 * n:128 * n + 128], (8, 128))
        oacc[n] = jnp.zeros((8, 128), F32)
    for half in range(2):
        issue_k(half)
        wait(big.at[pl.ds(SLOT * (NP - 2 + half), 60)], sems.at[1 + half])
        unpair_wq(half)
    issue_v_wo(0)
    wait_k(0)

    def slot_at(i):
        return bigw.at[pl.ds(SLOT * i, SLOT)]

    def layer(li, carry):
        first = li == 0
        ds, inv = layernorm([xres[n] for n in range(5)])
        for t in range(5):
            ylhs[t] = _rnd(ds[t] * inv)
        weave(chain(q_proj(slot_at(NP - 2), q0), q_proj(slot_at(NP - 1), q1),
                    scores(q0, 0, bigw, K0, s0), softmax(0, s0, p0),
                    scores(q0, 1, bigw, K0 + HS, s1)))
        linv[1] = jnp.zeros((8, 128), F32)
        zbuf[:, 0:2 * HS] = jnp.zeros((2, 2 * HS, 8, 128), F32)

        def step(i, c):
            @pl.when(first)
            def _():
                @pl.when(i < NP - 2)
                def _():
                    issue_k(i + 2)
                issue_v_wo(i + 1)

                @pl.when(i == NP - 2)
                def _():
                    issue_weight(w1_hbm, 0, w1b, 0, 30, sems.at[1])
                wait_k(i + 1)
                wait_v_wo(i)
                widen_v(i)

            h = 2 * i
            kv = bigw.at[pl.ds(SLOT * i, SLOT + 2 * HS)]
            prev = jnp.maximum(h - 2, 0)
            weave(chain(finish_step(prev), softmax(h + 1, s1, p1), pv_vpu(kv, range(HS), p0),
                        softmax(h + 2, s0, p0), pv_vpu(kv, range(HS, 2 * HS), p1)),
                  chain(scores(q1, 0, kv, SLOT, s0), scores(q1, 1, kv, SLOT + HS, s1),
                        q_proj(kv, q1), o_proj(kv)))
            return c

        lax.fori_loop(0, NP - 1, step, 0)

        @pl.when(first)
        def _():
            issue_weight(w2_hbm, 0, w2b, 0, 26, sems.at[2])
            issue_weight(w2_hbm, 26, w2b, 26, 4, sems.at[0])
            wait_v_wo(NP - 1)
            widen_v(NP - 1, 32)

        kv, last = slot_at(NP - 1), []
        weave(chain(softmax(H - 1, s1, p1), finish_step(H - 4), [300],
                    pv_mxu(kv, 32, p1, last), pv_mxu(kv, 40, p1, last), o_proj(kv)),
              chain(pv_vpu(kv, range(HS), p0, 2 * HS), pv_vpu(kv, range(HS, 32), p1, 2 * HS)))
        cols = lanes_to_cols(range(2 * HS, 2 * HS + 32))
        finish(H - 2, [all_rows_sum(cols[3]), all_rows_sum(cols[4]),
                       jnp.where(lane < 64, last[0], last[1])])
        weave(o_proj(slot_at(0)))

        @pl.when(first)
        def _():
            weave(ffn(wait))
        return carry

    def ffn(arrived):
        ds, inv = layernorm(residual())
        for t in range(10):
            ylhs[t] = jnp.where(same_c, _rnd(expand(ds[t // 2], t % 2) * inv), 0.0)
        arrived(w1b, sems.at[1])
        b1 = b1b[...].astype(F32)
        for j in range(6):
            hid = jnp.where(sub < 4, bcast_row(b1, 2 * j), bcast_row(b1, 2 * j + 1))
            for t in range(10):
                hid += mm(ylhs[t], vregs_of(w1w, [6 * i + j for i in range(8 * t, 8 * t + 8)]))
            for c, v in enumerate(halves(_rnd(jax.nn.gelu(hid, approximate=True)))):
                hlhs[2 * j + c] = down_lhs(v)
        arrived(w2b.at[0:26], sems.at[2])
        yield from down_proj(hlhs, range(10), w2w, 0, 16)
        arrived(w2b.at[26:30], sems.at[0])
        yield from down_proj(hlhs, range(10, 12), w2w, 0, 16)
        residual(b2b[...].astype(F32))

    lax.fori_loop(0, 2, layer, 0)
    weave(ffn(lambda ref, sem: None))
    out_ref[...] = jnp.concatenate([xres[n, 0:1, :] for n in range(5)], axis=1).astype(out_ref.dtype)


@jax.jit
def pallas_interleave_layers__sliding_block_cached__dense_activation_gelu__decode_kernel(
    A_x: jax.Array,
    A_k_cache: jax.Array,
    A_v_cache: jax.Array,
    A_wq: jax.Array,
    A_wo: jax.Array,
    B_x: jax.Array,
    B_w1: jax.Array,
    B_b1: jax.Array,
    B_w2: jax.Array,
    B_b2: jax.Array,
):
    del B_x
    cache = lambda a: _tile_order(jnp.transpose(a, (0, 1, 3, 2)).reshape(H * DH, SK), SK // 16)
    args = (
        A_x.reshape(1, D), cache(A_k_cache), cache(A_v_cache),
        _tile_order(A_wq, 256), _tile_order(A_wo, 240),
        _tile_order(B_w1, 256), B_b1.reshape(F // 128, 128),
        _tile_order(B_w2, 256), B_b2.reshape(D // 128, 128),
    )
    vm = pltpu.VMEM
    vregs = lambda *n: vm((*n, 8, 128), F32)
    out = pl.pallas_call(
        _kernel,
        out_shape=jax.ShapeDtypeStruct((1, D), A_x.dtype),
        in_specs=[pl.BlockSpec(memory_space=pl.ANY)] * len(args),
        scratch_shapes=[
            vm((NP * SLOT, WROWS, 128), BF16),
            vm((30, WROWS, 128), BF16), vm((30, WROWS, 128), BF16),
            vm((1, D), BF16), vm((F // 128, 128), BF16), vm((D // 128, 128), BF16),
            vregs(5), vregs(10), vregs(12), vregs(6), vregs(6), vregs(NJ + 1), vregs(NJ + 1),
            vregs(NJ), vregs(NJ), vregs(H), vregs(2, 2 * HS + 32), vregs(3), vregs(5),
            vm((8, 128), I32),
            pltpu.SemaphoreType.DMA((3,)), pltpu.SemaphoreType.DMA((2,)),
            pltpu.SemaphoreType.DMA((2,)), pltpu.SemaphoreType.DMA((2,)),
        ],
        compiler_params=pltpu.CompilerParams(vmem_limit_bytes=127 * 2 ** 20),
        name="interleave_decode",
    )(*args)
    return out.reshape(1, 1, D)
```
